```python
import jax
import jax.numpy as jnp

def _softmax(x, axis=-1):
    return jax.nn.softmax(x, axis=axis)
def _gelu(x):
    return jax.nn.gelu(x, approximate=True)
def _silu(x):
    return jax.nn.silu(x)
def _sigmoid(x):
    return jax.nn.sigmoid(x)
def _layernorm(x, axis=-1, eps=1e-5):
    m = jnp.mean(x, axis=axis, keepdims=True)
    v = jnp.var(x, axis=axis, keepdims=True)
    return (x - m) / jnp.sqrt(v + eps)
def _scatter_add(tgt, idx, src, axis=0):
    return tgt.at[idx].add(src)
def _segment_sum(src, seg, n):
    return jax.ops.segment_sum(src, seg, n)
class _Rng:
    def __init__(self, key):
        self._k = key
    def _next(self):
        self._k, sub = jax.random.split(self._k)
        return sub
    def normal(self, shape):
        return jax.random.normal(self._next(), shape, dtype=jnp.bfloat16)
    def randint(self, lo, hi, shape):
        return jax.random.randint(self._next(), shape, lo, hi, dtype=jnp.int32)
    def uniform(self, shape, lo=0.0, hi=1.0):
        return jax.random.uniform(self._next(), shape, jnp.bfloat16, lo, hi)
    def permutation(self, n):
        return jax.random.permutation(self._next(), n)


kernel_name = 'recurrent_scan__linear_kernel_hedgehog__dense_activation_relu__prompt'

def _fwd_setup_inputs():
    _rng = _Rng(jax.random.key(int.from_bytes(__import__("os").urandom(4), "little")))
    _w = (lambda a: (lambda t: t.astype(jnp.bfloat16) if jnp.issubdtype(t.dtype, jnp.floating) else t)(jnp.asarray(a)))
    def _A_setup():
        B, S, D, H = 1, 2048, 1024, 32
        Dh = D // H
        return {
            "x": _w((lambda *s: _rng.normal(s) * 0.05)(B, S, D)),
            "wqkv": _w((lambda *s: _rng.normal(s) * 0.05)(D, 3 * D)),
            "w_phi": _w((lambda *s: _rng.normal(s) * 0.05)(H, Dh, Dh) * (Dh ** -0.5)),
            "wo": _w((lambda *s: _rng.normal(s) * 0.05)(D, D)),
        }
    _A_in = _A_setup()

    def _B_setup():
        B, S, D, Dff = 1, 2048, 1024, 3584
        return {
            "x": _w((lambda *s: _rng.normal(s) * 0.05)(B, S, D)),
            "w1": _w((lambda *s: _rng.normal(s) * 0.05)(D, Dff)),
            "w2": _w((lambda *s: _rng.normal(s) * 0.05)(Dff, D)),
        }
    _B_in = _B_setup()

    return {
        "A_x": _A_in["x"],
        "A_wqkv": _A_in["wqkv"],
        "A_w_phi": _A_in["w_phi"],
        "A_wo": _A_in["wo"],
        "B_x": _B_in["x"],
        "B_w1": _B_in["w1"],
        "B_w2": _B_in["w2"],
    }

def _fwd_reference(A_x, A_wqkv, A_w_phi, A_wo, B_x, B_w1, B_w2):
    def _A_ref(x, wqkv, w_phi, wo):
        B, S, D = x.shape
        H = 32; Dh = D // H
        qkv = (lambda x, *d: x.transpose(*d))((x @ wqkv).reshape(B, S, 3, H, Dh), 2, 0, 3, 1, 4)
        q, k, v = qkv[0], qkv[1], qkv[2]
        pq = jnp.einsum("bhsd,hdf->bhsf", q, w_phi)
        pk = jnp.einsum("bhsd,hdf->bhsf", k, w_phi)
        phi_q = jnp.concatenate([_softmax(pq, axis=-1), _softmax(-pq, axis=-1)], axis=-1)
        phi_k = jnp.concatenate([_softmax(pk, axis=-1), _softmax(-pk, axis=-1)], axis=-1)
        kv = jnp.einsum("bhsf,bhsd->bhfd", phi_k, v)
        z  = jnp.einsum("bhsf->bhf", phi_k)
        num = jnp.einsum("bhqf,bhfd->bhqd", phi_q, kv)
        den = jnp.einsum("bhqf,bhf->bhq", phi_q, z)[..., None] + 1e-6
        o = num / den
        return (lambda x, *d: x.transpose(*d))(o, 0, 2, 1, 3).reshape(B, S, D) @ wo

    def _B_ref(x, w1, w2):
        h = jnp.einsum("bsd,df->bsf", x, w1)
        zero = jnp.zeros_like(h)
        h = jnp.maximum(h, zero)
        return jnp.einsum("bsf,fd->bsd", h, w2)

    x = A_x
    xn = _layernorm(x, axis=-1)
    s = _A_ref(xn, A_wqkv, A_w_phi, A_wo)
    g = _silu(_B_ref(xn, B_w1, B_w2))
    return x + s * g


def setup_inputs():
    _inp = _fwd_setup_inputs()
    _gk = jax.random.fold_in(jax.random.key(int.from_bytes(__import__("os").urandom(4), "little")), 2**31 - 1)
    _shapes = [[1, 2048, 1024]]
    _dtypes = ['bfloat16']
    _gks = jax.random.split(_gk, len(_shapes))
    _gs = [jax.random.normal(k, s, dtype=jnp.dtype(d)) * 0.05 for k, s, d in zip(_gks, _shapes, _dtypes)]
    _inp["grad_out"] = _gs[0]
    return _inp

def reference(A_x, A_wqkv, A_w_phi, A_wo, B_w1, B_w2, B_x, grad_out):
    _const = dict(B_x=B_x)
    def _f(*_d):
        return _fwd_reference(**{'A_x': _d[0], 'A_wqkv': _d[1], 'A_w_phi': _d[2], 'A_wo': _d[3], 'B_w1': _d[4], 'B_w2': _d[5], **_const})
    _out, _vjp = jax.vjp(_f, A_x, A_wqkv, A_w_phi, A_wo, B_w1, B_w2)
    _grads = _vjp(grad_out)
    _out0 = jnp.asarray(_out)
    return (_out0, *[jnp.asarray(_g) for _g in _grads])
```

```python
import jax
import jax.numpy as jnp
from jax import lax
import jax.experimental.pallas as pl
import jax.experimental.pallas.tpu as pltpu

S, D, H, DH, F = 2048, 1024, 32, 32, 3584
T = 256
NT = S // T
NG = 8
AR = 160
F32 = jnp.float32
BF16 = jnp.bfloat16

_NN = (((1,), (0,)), ((), ()))
_NTD = (((1,), (1,)), ((), ()))
_TN = (((0,), (0,)), ((), ()))


def _dot(a, b, dims=_NN):
    return lax.dot_general(a, b, dims, preferred_element_type=F32)


def _softmax_pm(pT):
    p4 = pT.reshape(NG, 16, 8, T)
    mx = jnp.max(p4, axis=1)
    mx = jnp.maximum(mx, pltpu.roll(mx, 4, 1))
    mn = jnp.min(p4, axis=1)
    mn = jnp.minimum(mn, pltpu.roll(mn, 4, 1))
    ep = jnp.exp(p4 - mx[:, None])
    em = jnp.exp(mn[:, None] - p4)
    sp = jnp.sum(ep, axis=1)
    sp = sp + pltpu.roll(sp, 4, 1)
    sm = jnp.sum(em, axis=1)
    sm = sm + pltpu.roll(sm, 4, 1)
    ap = ep * (1.0 / sp)[:, None]
    am = em * (1.0 / sm)[:, None]
    return ap, am


def _softmax_pm_bwd(ap, am, dap, dam):
    cp = jnp.sum(ap * dap, axis=0)
    cp = cp + pltpu.roll(cp, 4, 0)
    cm = jnp.sum(am * dam, axis=0)
    cm = cm + pltpu.roll(cm, 4, 0)
    dp = ap * (dap - cp[None]) - am * (dam - cm[None])
    return dp.reshape(128, T)


def _head_mask():
    row = lax.broadcasted_iota(jnp.int32, (AR, 256), 0)
    col = lax.broadcasted_iota(jnp.int32, (AR, 256), 1)
    rh = jnp.where(row < 128, row // 32, (row - 128) // 8)
    return rh == (col % 4)


def _kernel(x_hbm, wqkv_hbm, wphi_ref, wo_hbm, w1_hbm, w2_hbm, dy_hbm,
            out_hbm, dx_hbm, dwqkv_hbm, dwphi_ref, dwo_hbm, dw1_hbm, dw2_hbm,
            x_v, dy_v, wall_v, wt_v, wo_v, w1_v, w2_v, wbd_v,
            xnT_v, rstd_v, phik_v, vT_v, hT_v, dhp_v, df_v, oT_v, ds_v, dpqT_v,
            acc_v, abf_v, kv_v, zb_v, g_v,
            in_sems, out_sems):
    cp_x = pltpu.make_async_copy(x_hbm, x_v, in_sems.at[0])
    cp_wqkv = pltpu.make_async_copy(wqkv_hbm, wall_v, in_sems.at[1])
    cp_w1 = pltpu.make_async_copy(w1_hbm, w1_v, in_sems.at[2])
    cp_w2 = pltpu.make_async_copy(w2_hbm, w2_v, in_sems.at[3])
    cp_wo = pltpu.make_async_copy(wo_hbm, wo_v, in_sems.at[4])
    cp_dy = pltpu.make_async_copy(dy_hbm, dy_v, in_sems.at[5])
    cp_wqkv.start()
    cp_x.start()
    cp_w1.start()
    cp_wo.start()
    cp_w2.start()
    cp_dy.start()

    e_r = lax.broadcasted_iota(jnp.int32, (DH, 128), 0)
    e_c = lax.broadcasted_iota(jnp.int32, (DH, 128), 1)
    expand = jnp.where(e_c // 4 == e_r, 1.0, 0.0).astype(BF16)
    wexp = _dot(wphi_ref[...], expand)
    b_r = lax.broadcasted_iota(jnp.int32, (D, 128), 0)
    b_c = lax.broadcasted_iota(jnp.int32, (D, 128), 1)
    wbd_v[...] = jnp.where((b_r // 32) % 4 == b_c % 4, wexp, 0.0).astype(BF16)

    cp_wqkv.wait()
    for j in range(2 * NG):
        g = j % NG
        cols = slice(j * 128, (j + 1) * 128)
        wall_v[:, cols] = _dot(wall_v[:, cols], wbd_v[g * 128:(g + 1) * 128, :]).astype(BF16)
    for j in range(3 * NG):
        wt_v[j * 128:(j + 1) * 128, :] = wall_v[:, j * 128:(j + 1) * 128].T

    acc_v[...] = jnp.zeros(acc_v.shape, F32)
    ones_rows = jnp.ones((AR - 128, T), BF16)
    cp_x.wait()

    def p1(t, carry):
        r0 = pl.multiple_of(t * T, T)
        rows = pl.ds(r0, T)
        x = x_v[rows, :].astype(F32)
        mu = jnp.mean(x, axis=1, keepdims=True)
        xc = x - mu
        var = jnp.mean(xc * xc, axis=1, keepdims=True)
        rstd = lax.rsqrt(var + 1e-5)
        xn = (xc * rstd).astype(BF16)
        rstd_v[rows, :] = jnp.broadcast_to(rstd, (T, 128))
        xnT = xn.T
        xnT_v[:, rows] = xnT
        pkT = _dot(wt_v[D:2 * D, :], xnT)
        vT = _dot(wt_v[2 * D:3 * D, :], xnT).astype(BF16)
        vT_v[:, rows] = vT
        ap, am = _softmax_pm(pkT)
        apb = ap.reshape(NG, 128, T).astype(BF16)
        amb = am.reshape(NG, 128, T).astype(BF16)
        phik_v[:, 0:128, rows] = apb
        phik_v[:, 128:256, rows] = amb
        for g in range(NG):
            lhs = jnp.concatenate([vT[g * 128:(g + 1) * 128], ones_rows], axis=0)
            rhs = jnp.concatenate([apb[g], amb[g]], axis=0)
            acc_v[g] += _dot(lhs, rhs, _NTD)
        return carry

    lax.fori_loop(0, NT, p1, 0)

    mask = _head_mask()
    for g in range(NG):
        a = acc_v[g]
        am_ = jnp.where(mask, a, 0.0)
        abf_v[g] = am_.astype(BF16)
        kv_v[g] = am_[0:128].T.astype(BF16)
        zb_v[g] = jnp.tile(a[128:136], (16, 1)).T
    acc_v[...] = jnp.zeros(acc_v.shape, F32)

    cp_w1.wait()
    cp_wo.wait()
    cp_w2.wait()
    cp_dy.wait()

    sub4 = lax.broadcasted_iota(jnp.int32, (NG, 8, T), 1) % 4

    def p2(t, carry):
        r0 = pl.multiple_of(t * T, T)
        rows = pl.ds(r0, T)
        xnT = xnT_v[:, rows]
        pqT = _dot(wt_v[0:D, :], xnT)
        ap, am = _softmax_pm(pqT)
        apb = ap.reshape(NG, 128, T).astype(BF16)
        amb = am.reshape(NG, 128, T).astype(BF16)
        phiq = [jnp.concatenate([apb[g], amb[g]], axis=0) for g in range(NG)]
        nd = [_dot(abf_v[g], phiq[g]) for g in range(NG)]
        num = jnp.concatenate([n[0:128] for n in nd], axis=0).reshape(H, 4, 8, T)
        den = jnp.concatenate([n[128:AR] for n in nd], axis=0).reshape(H, 8, T) + 1e-6
        rden = 1.0 / den
        oT4 = num * rden[:, None]
        oTb = oT4.reshape(D, T).astype(BF16)
        oT_v[:, rows] = oTb
        s = _dot(oTb, wo_v[...], _TN)

        pre = _dot(xnT, w1_v[...], _TN)
        h = jnp.maximum(pre, 0.0).astype(BF16)
        hT_v[:, rows] = h.T
        f = _dot(h, w2_v[...])
        sig = 1.0 / (1.0 + jnp.exp(-f))
        gate = f * sig
        x = x_v[rows, :].astype(F32)
        dy = dy_v[rows, :].astype(F32)
        x_v[rows, :] = (x + s * gate).astype(BF16)
        pltpu.make_async_copy(x_v.at[rows, :], out_hbm.at[rows, :], out_sems.at[t]).start()
        ds = (dy * gate).astype(BF16)
        ds_v[rows, :] = ds
        df = (dy * s * (sig * (1.0 + f * (1.0 - sig)))).astype(BF16)
        df_v[rows, :] = df

        dh = _dot(df, w2_v[...], _NTD)
        dhp = jnp.where(pre > 0.0, dh, jnp.where(pre == 0.0, 0.5 * dh, 0.0))
        dhp_v[rows, :] = dhp.astype(BF16)

        doT4 = _dot(wo_v[...], ds, _NTD).reshape(H, 4, 8, T)
        dnumb = (doT4 * rden[:, None]).reshape(D, T).astype(BF16)
        tt = jnp.sum(doT4 * oT4, axis=1)
        tt = tt + pltpu.roll(tt, 4, 1)
        tt = tt + pltpu.roll(tt, 2, 1)
        tt = tt + pltpu.roll(tt, 1, 1)
        dd = -(tt * rden)
        ddb = dd.reshape(H * 8, T).astype(BF16)
        dd4 = dd.reshape(NG, 4, 8, T)
        dd8 = jnp.where(sub4 == 0, dd4[:, 0],
                        jnp.where(sub4 == 1, dd4[:, 1],
                                  jnp.where(sub4 == 2, dd4[:, 2], dd4[:, 3])))
        for g in range(NG):
            dn = dnumb[g * 128:(g + 1) * 128]
            dphi = _dot(kv_v[g], dn).reshape(32, 8, T)
            dphi = dphi + jnp.tile(zb_v[g], (1, T // 128)).reshape(32, 8, T) * dd8[g][None]
            dp = _softmax_pm_bwd(ap[g], am[g], dphi[0:16], dphi[16:32])
            dpqT_v[g * 128:(g + 1) * 128, rows] = dp.astype(BF16)
            lhs = jnp.concatenate([dn, ddb[g * 32:(g + 1) * 32]], axis=0)
            acc_v[g] += _dot(lhs, phiq[g], _NTD)
        return carry

    lax.fori_loop(0, NT, p2, 0)

    cp_wq = pltpu.make_async_copy(wqkv_hbm.at[:, 0:D], wt_v.at[0:D, :], in_sems.at[6])
    cp_wk = pltpu.make_async_copy(wqkv_hbm.at[:, D:2 * D], wt_v.at[D:2 * D, :], in_sems.at[7])
    cp_wq.start()
    cp_wk.start()

    for g in range(NG):
        a = jnp.where(mask, acc_v[g], 0.0)
        abf_v[g] = a.astype(BF16)
        kv_v[g] = a[0:128].T.astype(BF16)
        dz = a[128:136] + a[136:144] + a[144:152] + a[152:160]
        zb_v[g] = jnp.tile(dz, (16, 1)).T

    C2 = 512

    def dw2_body(c, carry):
        rr = pl.ds(pl.multiple_of(c * C2, C2), C2)
        w2_v[rr, :] = _dot(hT_v[rr, :], df_v[...]).astype(BF16)
        pltpu.make_async_copy(w2_v.at[rr, :], dw2_hbm.at[rr, :], out_sems.at[16 + c]).start()
        return carry

    lax.fori_loop(0, F // C2, dw2_body, 0)

    def dwo_body(c, carry):
        rr = pl.ds(pl.multiple_of(c * C2, C2), C2)
        wo_v[rr, :] = _dot(oT_v[rr, :], ds_v[...]).astype(BF16)
        pltpu.make_async_copy(wo_v.at[rr, :], dwo_hbm.at[rr, :], out_sems.at[24 + c]).start()
        return carry

    lax.fori_loop(0, D // C2, dwo_body, 0)

    def p3(t, carry):
        r0 = pl.multiple_of(t * T, T)
        rows = pl.ds(r0, T)
        dpk = []
        dv = []
        for g in range(NG):
            phk = phik_v[g, :, rows]
            dphi = _dot(kv_v[g], vT_v[g * 128:(g + 1) * 128, rows])
            dphi = (dphi + jnp.tile(zb_v[g], (1, T // 128))).reshape(32, 8, T)
            a = phk.astype(F32).reshape(32, 8, T)
            dpk.append(_softmax_pm_bwd(a[0:16], a[16:32], dphi[0:16], dphi[16:32]).astype(BF16))
            dv.append(_dot(abf_v[g, 0:128, :], phk).astype(BF16))
        dpkT = jnp.concatenate(dpk, axis=0)
        dvT = jnp.concatenate(dv, axis=0)
        oT_v[:, rows] = dpkT
        vT_v[:, rows] = dvT
        dxnT = (_dot(w1_v[...], dhp_v[rows, :], _NTD)
                + _dot(wall_v[:, 0:D], dpqT_v[:, rows])
                + _dot(wall_v[:, D:2 * D], dpkT)
                + _dot(wall_v[:, 2 * D:3 * D], dvT))
        xnT = xnT_v[:, rows].astype(F32)
        m1 = jnp.mean(dxnT, axis=0, keepdims=True)
        m2 = jnp.mean(dxnT * xnT, axis=0, keepdims=True)
        u = dxnT - m1 - xnT * m2
        dx = dy_v[rows, :].astype(F32) + jnp.tile(rstd_v[rows, :], (1, D // 128)) * u.T
        dy_v[rows, :] = dx.astype(BF16)
        pltpu.make_async_copy(dy_v.at[rows, :], dx_hbm.at[rows, :], out_sems.at[8 + t]).start()
        return carry

    lax.fori_loop(0, NT, p3, 0)

    C1 = 256

    def dw1_body(c, carry):
        rr = pl.ds(pl.multiple_of(c * C1, C1), C1)
        w1_v[rr, :] = _dot(xnT_v[rr, :], dhp_v[...]).astype(BF16)
        pltpu.make_async_copy(w1_v.at[rr, :], dw1_hbm.at[rr, :], out_sems.at[26 + c]).start()
        return carry

    lax.fori_loop(0, D // C1, dw1_body, 0)

    def g_body(c, carry):
        rr = pl.ds(pl.multiple_of(c * C1, C1), C1)
        xr = xnT_v[rr, :]
        gq = _dot(xr, dpqT_v[...], _NTD).astype(BF16)
        gk = _dot(xr, oT_v[...], _NTD).astype(BF16)
        g_v[rr, 0:D] = gq
        g_v[rr, D:2 * D] = gk
        wall_v[rr, 2 * D:3 * D] = _dot(xr, vT_v[...], _NTD).astype(BF16)
        for g in range(NG):
            wb = wbd_v[g * 128:(g + 1) * 128, :]
            wall_v[rr, g * 128:(g + 1) * 128] = _dot(gq[:, g * 128:(g + 1) * 128], wb, _NTD).astype(BF16)
            wall_v[rr, D + g * 128:D + (g + 1) * 128] = _dot(gk[:, g * 128:(g + 1) * 128], wb, _NTD).astype(BF16)
        pltpu.make_async_copy(wall_v.at[rr, :], dwqkv_hbm.at[rr, :], out_sems.at[30 + c]).start()
        return carry

    lax.fori_loop(0, D // C1, g_body, 0)

    cp_wq.wait()
    cp_wk.wait()
    m_r = lax.broadcasted_iota(jnp.int32, (128, 128), 0)
    m_c = lax.broadcasted_iota(jnp.int32, (128, 128), 1)
    bmask = (m_r // 32) == (m_c % 4)
    for g in range(NG):
        cq = slice(g * 128, (g + 1) * 128)
        ck = slice(D + g * 128, D + (g + 1) * 128)
        m = _dot(wt_v[0:D, cq], g_v[:, cq], _TN) + _dot(wt_v[D:2 * D, cq], g_v[:, ck], _TN)
        mb = jnp.where(bmask, m, 0.0).astype(BF16)
        dwphi_ref[cq, :] = _dot(mb, expand, _NTD).astype(BF16)

    for t in range(NT):
        rows = pl.ds(t * T, T)
        pltpu.make_async_copy(x_v.at[rows, :], out_hbm.at[rows, :], out_sems.at[t]).wait()
        pltpu.make_async_copy(dy_v.at[rows, :], dx_hbm.at[rows, :], out_sems.at[8 + t]).wait()
    for c in range(F // C2):
        rr = pl.ds(c * C2, C2)
        pltpu.make_async_copy(w2_v.at[rr, :], dw2_hbm.at[rr, :], out_sems.at[16 + c]).wait()
    for c in range(D // C2):
        rr = pl.ds(c * C2, C2)
        pltpu.make_async_copy(wo_v.at[rr, :], dwo_hbm.at[rr, :], out_sems.at[24 + c]).wait()
    for c in range(D // C1):
        rr = pl.ds(c * C1, C1)
        pltpu.make_async_copy(w1_v.at[rr, :], dw1_hbm.at[rr, :], out_sems.at[26 + c]).wait()
        pltpu.make_async_copy(wall_v.at[rr, :], dwqkv_hbm.at[rr, :], out_sems.at[30 + c]).wait()


@jax.jit
def pallas_recurrent_scan__linear_kernel_hedgehog__dense_activation_relu__prompt_kernel(
    A_x: jax.Array,
    A_wqkv: jax.Array,
    A_w_phi: jax.Array,
    A_wo: jax.Array,
    B_x: jax.Array,
    B_w1: jax.Array,
    B_w2: jax.Array,
    grad_out: jax.Array,
):
    del B_x
    x = A_x.reshape(S, D)
    dy = grad_out.reshape(S, D)
    wphi = A_w_phi.reshape(H * DH, DH)
    any_spec = pl.BlockSpec(memory_space=pl.ANY)
    vmem_spec = pl.BlockSpec(memory_space=pltpu.VMEM)
    out_shape = (
        jax.ShapeDtypeStruct((S, D), BF16),
        jax.ShapeDtypeStruct((S, D), BF16),
        jax.ShapeDtypeStruct((D, 3 * D), BF16),
        jax.ShapeDtypeStruct((H * DH, DH), BF16),
        jax.ShapeDtypeStruct((D, D), BF16),
        jax.ShapeDtypeStruct((D, F), BF16),
        jax.ShapeDtypeStruct((F, D), BF16),
    )
    scratch = [
        pltpu.VMEM((S, D), BF16),
        pltpu.VMEM((S, D), BF16),
        pltpu.VMEM((D, 3 * D), BF16),
        pltpu.VMEM((3 * D, D), BF16),
        pltpu.VMEM((D, D), BF16),
        pltpu.VMEM((D, F), BF16),
        pltpu.VMEM((F, D), BF16),
        pltpu.VMEM((D, 128), BF16),
        pltpu.VMEM((D, S), BF16),
        pltpu.VMEM((S, 128), F32),
        pltpu.VMEM((NG, 256, S), BF16),
        pltpu.VMEM((D, S), BF16),
        pltpu.VMEM((F, S), BF16),
        pltpu.VMEM((S, F), BF16),
        pltpu.VMEM((S, D), BF16),
        pltpu.VMEM((D, S), BF16),
        pltpu.VMEM((S, D), BF16),
        pltpu.VMEM((D, S), BF16),
        pltpu.VMEM((NG, AR, 256), F32),
        pltpu.VMEM((NG, AR, 256), BF16),
        pltpu.VMEM((NG, 256, 128), BF16),
        pltpu.VMEM((NG, 256, 128), F32),
        pltpu.VMEM((D, 2 * D), BF16),
        pltpu.SemaphoreType.DMA((8,)),
        pltpu.SemaphoreType.DMA((34,)),
    ]
    outs = pl.pallas_call(
        _kernel,
        out_shape=out_shape,
        in_specs=[any_spec, any_spec, vmem_spec, any_spec, any_spec, any_spec, any_spec],
        out_specs=(any_spec, any_spec, any_spec, vmem_spec, any_spec, any_spec, any_spec),
        scratch_shapes=scratch,
        compiler_params=pltpu.CompilerParams(vmem_limit_bytes=124 * 1024 * 1024),
    )(x, A_wqkv, wphi, A_wo, B_w1, B_w2, dy)
    out, dx, dwqkv, dwphi, dwo, dw1, dw2 = outs
    return (out.reshape(1, S, D), dx.reshape(1, S, D), dwqkv, dwphi.reshape(H, DH, DH), dwo, dw1, dw2)
```

```python
import jax
import jax.numpy as jnp
from jax import lax
import jax.experimental.pallas as pl
import jax.experimental.pallas.tpu as pltpu

S, D, H, DH, F = 2048, 1024, 32, 32, 3584
T = 256
NT = S // T
NP = 16
AR = 80
F32 = jnp.float32
BF16 = jnp.bfloat16

_NN = (((1,), (0,)), ((), ()))
_NTD = (((1,), (1,)), ((), ()))
_TN = (((0,), (0,)), ((), ()))


def _dot(a, b, dims=_NN):
    return lax.dot_general(a, b, dims, preferred_element_type=F32)


def _fold(x, op, axis):
    x = op(x, pltpu.roll(x, 4, axis))
    return op(x, pltpu.roll(x, 2, axis))


def _softmax_pm(pT):
    p4 = pT.reshape(NP, 8, 8, T)
    mx = _fold(jnp.max(p4, axis=1), jnp.maximum, 1)
    mn = _fold(jnp.min(p4, axis=1), jnp.minimum, 1)
    ep = jnp.exp(p4 - mx[:, None])
    em = jnp.exp(mn[:, None] - p4)
    sp = _fold(jnp.sum(ep, axis=1), jnp.add, 1)
    sm = _fold(jnp.sum(em, axis=1), jnp.add, 1)
    ap = ep * (1.0 / sp)[:, None]
    am = em * (1.0 / sm)[:, None]
    return ap.reshape(NP, 64, T).astype(BF16), am.reshape(NP, 64, T).astype(BF16)


def _softmax_pm_bwd(a, da):
    a4 = a.reshape(2, 8, 8, T)
    da4 = da.reshape(2, 8, 8, T)
    c = _fold(jnp.sum(a4 * da4, axis=1), jnp.add, 1)
    r = a4 * (da4 - c[:, None])
    return (r[0] - r[1]).reshape(64, T)


def _pair_mask():
    row = lax.broadcasted_iota(jnp.int32, (AR, 128), 0)
    col = lax.broadcasted_iota(jnp.int32, (AR, 128), 1)
    rh = jnp.where(row < 64, row // 32, (row - 64) // 8)
    return rh == (col % 2)


def _kernel(x_hbm, wqkv_hbm, wphi_ref, wo_hbm, w1_hbm, w2_hbm, dy_hbm,
            out_hbm, dx_hbm, dwqkv_hbm, dwphi_ref, dwo_hbm, dw1_hbm, dw2_hbm,
            x_v, dy_v, wall_v, wt_v, wo_v, w1_v, w2_v, wbd_v,
            xnT_v, rstd_v, phik_v, phiq_v, vT_v, hT_v, dhp_v, df_v, oT_v, ds_v, gate_v,
            acc_v, abf_v, at_v, m_v, dxn_v,
            in_sems, x_sems, w_sems, out_sems):
    def x_copy(t):
        rows = pl.ds(pl.multiple_of(t * T, T), T)
        return pltpu.make_async_copy(x_hbm.at[rows, :], x_v.at[rows, :], x_sems.at[t])

    def w_copy(j):
        r = pl.ds(pl.multiple_of(j * 128, 128), 128)
        return pltpu.make_async_copy(wqkv_hbm.at[r, :], wall_v.at[r, :], w_sems.at[j])

    cp_w1 = pltpu.make_async_copy(w1_hbm, w1_v, in_sems.at[3])
    cp_w2 = pltpu.make_async_copy(w2_hbm, w2_v, in_sems.at[4])
    cp_wo = pltpu.make_async_copy(wo_hbm, wo_v, in_sems.at[5])
    cp_dy = pltpu.make_async_copy(dy_hbm, dy_v, in_sems.at[6])
    x_copy(0).start()
    w_copy(0).start()

    e_r = lax.broadcasted_iota(jnp.int32, (DH, 128), 0)
    e_c = lax.broadcasted_iota(jnp.int32, (DH, 128), 1)
    expand = jnp.where((e_c % 64) // 2 == e_r, 1.0, 0.0).astype(BF16)
    wexp = _dot(wphi_ref[...], expand)
    b_r = lax.broadcasted_iota(jnp.int32, (D, 128), 0)
    b_c = lax.broadcasted_iota(jnp.int32, (D, 128), 1)
    wbd_v[...] = jnp.where((b_r // 32) % 4 == (b_c // 64) * 2 + b_c % 2, wexp, 0.0).astype(BF16)
    acc_v[...] = jnp.zeros(acc_v.shape, F32)

    def layernorm(t, pace=None):
        rows = pl.ds(pl.multiple_of(t * T, T), T)
        x = x_v[rows, :].astype(F32)
        if pace is not None:
            x = pace(x)
        mu = jnp.mean(x, axis=1, keepdims=True)
        xc = x - mu
        var = jnp.mean(xc * xc, axis=1, keepdims=True)
        rstd = lax.rsqrt(var + 1e-5)
        rstd_v[rows, :] = jnp.broadcast_to(rstd, (T, 128))
        xn = (xc * rstd).astype(BF16)
        gate_v[rows, :] = xn
        xnT_v[:, rows] = xn.T

    w_copy(1).start()
    x_copy(0).wait()
    w_copy(2).start()
    layernorm(0)

    def start_body(i, carry):
        w_copy(i).wait()

        @pl.when(i < 5)
        def _():
            w_copy(i + 3).start()

        @pl.when(i >= 6)
        def _():
            x_copy(i - 5).start()

        r = pl.ds(pl.multiple_of(i * 128, 128), 128)
        w_in = wall_v[r, :]
        w = jnp.concatenate(
            [_dot(w_in[:, j * 128:(j + 1) * 128], wbd_v[(j % 8) * 128:(j % 8 + 1) * 128, :]).astype(BF16)
             for j in range(16)] + [w_in[:, 2 * D:3 * D]], axis=1)
        wall_v[r, :] = w
        wt_v[:, r] = w.T
        return carry

    lax.fori_loop(0, 8, start_body, 0)
    for t in range(3, NT):
        x_copy(t).start()
    cp_w1.start()
    cp_w2.start()
    cp_dy.start()
    cp_wo.start()

    ones_rows = jnp.ones((AR - 64, T), BF16)

    def l1(t, carry):
        @pl.when(t + 1 < NT)
        def _():
            x_copy(t + 1).wait()

        rows = pl.ds(pl.multiple_of(t * T, T), T)
        never = (lax.broadcasted_iota(jnp.int32, (8, 128), 0) + t) < 0
        xnT = xnT_v[:, rows]
        vf = _dot(wt_v[2 * D:3 * D, :], xnT)
        kp, km = _softmax_pm(_dot(wt_v[D:2 * D, :], xnT))
        qp, qm = _softmax_pm(_dot(wt_v[0:D, :], xnT))
        vT = vf.astype(BF16)

        def pace(x):
            v4 = vf.reshape(T // 8, 4, 8, T)
            z = jnp.concatenate([v4[:, q] for q in range(4)], axis=2)
            m = jnp.tile(never, (1, D // 128))[None]
            return jnp.where(m, z, x.reshape(T // 8, 8, D)).reshape(T, D)

        layernorm(jnp.minimum(t + 1, NT - 1), pace)
        phik_v[:, 0:64, rows] = kp
        phik_v[:, 64:128, rows] = km
        phiq_v[:, 0:64, rows] = qp
        phiq_v[:, 64:128, rows] = qm
        vT_v[:, rows] = vT
        for p in range(NP):
            lhs = jnp.concatenate([vT[p * 64:(p + 1) * 64], ones_rows], axis=0)
            rhs = jnp.concatenate([kp[p], km[p]], axis=0)
            acc_v[p] += _dot(lhs, rhs, _NTD)
        return carry

    lax.fori_loop(0, NT, l1, 0)

    cp_wq = pltpu.make_async_copy(wqkv_hbm.at[:, 0:D], wt_v.at[0:D, :], in_sems.at[7])
    cp_wk = pltpu.make_async_copy(wqkv_hbm.at[:, D:2 * D], wt_v.at[D:2 * D, :], in_sems.at[8])
    cp_wq.start()
    cp_wk.start()

    zpad = jnp.zeros((128 - AR, 128), F32)

    def finalize():
        mask = _pair_mask()
        for p in range(NP):
            a = jnp.where(mask, acc_v[p], 0.0)
            abf_v[p] = a.astype(BF16)
            at_v[p] = jnp.concatenate([a, zpad], axis=0).T.astype(BF16)
        acc_v[...] = jnp.zeros(acc_v.shape, F32)

    finalize()

    cp_w1.wait()
    cp_w2.wait()
    cp_dy.wait()

    def lx(t, carry):
        rows = pl.ds(pl.multiple_of(t * T, T), T)
        pre = _dot(gate_v[rows, :], w1_v[...])
        h = jnp.where(pre == 0.0, -0.0, jnp.maximum(pre, 0.0)).astype(BF16)
        dhp_v[rows, :] = h
        hT_v[:, rows] = h.T
        f = _dot(h, w2_v[...])
        sig = 0.5 * jnp.tanh(0.5 * f) + 0.5
        gate = f * sig
        dy = dy_v[rows, :].astype(F32)
        gate_v[rows, :] = gate.astype(BF16)
        ds_v[rows, :] = (dy * gate).astype(BF16)
        df_v[rows, :] = (dy * (sig * (1.0 + f * (1.0 - sig)))).astype(BF16)
        return carry

    lax.fori_loop(0, NT, lx, 0)

    cp_wo.wait()
    zrows = jnp.zeros((128 - AR, T), BF16)

    def ly(t, carry):
        rows = pl.ds(pl.multiple_of(t * T, T), T)
        ds = ds_v[rows, :]
        phiq = [phiq_v[p, :, rows] for p in range(NP)]
        do4, o4, rd = [], [], []
        for c in range(8):
            for p in (2 * c, 2 * c + 1):
                n = _dot(abf_v[p], phiq[p])
                r = 1.0 / (n[64:AR].reshape(2, 8, T) + 1e-6)
                rd.append(r)
                o4.append(n[0:64].reshape(2, 4, 8, T) * r[:, None])
            d = _dot(wo_v[c * 128:(c + 1) * 128, :], ds, _NTD).reshape(2, 2, 4, 8, T)
            do4 += [d[0], d[1]]
        oTb = jnp.concatenate([o.reshape(64, T).astype(BF16) for o in o4], axis=0)
        oT_v[:, rows] = oTb
        o_n = oTb.T

        def attn_bwd(p):
            dn = (do4[p] * rd[p][:, None]).reshape(64, T).astype(BF16)
            tt = jnp.sum(do4[p] * o4[p], axis=1)
            tt = tt + pltpu.roll(tt, 4, 1)
            tt = tt + pltpu.roll(tt, 2, 1)
            tt = tt + pltpu.roll(tt, 1, 1)
            dd = (tt * rd[p] * (-0.125)).reshape(16, T).astype(BF16)
            lhs = jnp.concatenate([dn, dd], axis=0)
            dphi = _dot(at_v[p], jnp.concatenate([lhs, zrows], axis=0))
            dp = _softmax_pm_bwd(phiq[p].astype(F32), dphi)
            acc_v[p] += _dot(lhs, phiq[p], _NTD)
            phiq_v[p, 0:64, rows] = dp.astype(BF16)

        dfs = []
        for c in range(4):
            attn_bwd(c)
            cs = slice(c * 256, (c + 1) * 256)
            s = _dot(o_n, wo_v[:, cs])
            x_v[rows, cs] = (x_v[rows, cs].astype(F32) + s * gate_v[rows, cs].astype(F32)).astype(BF16)
            dfs.append((df_v[rows, cs].astype(F32) * s).astype(BF16))
        df = jnp.concatenate(dfs, axis=1)
        df_v[rows, :] = df
        pltpu.make_async_copy(x_v.at[rows, :], out_hbm.at[rows, :], out_sems.at[t]).start()

        for c in range(14):
            if c < 12:
                attn_bwd(4 + c)
            cs = slice(c * 256, (c + 1) * 256)
            dh = _dot(df, w2_v[cs, :], _NTD)
            hb = lax.bitcast_convert_type(dhp_v[rows, cs].astype(F32), jnp.int32)
            dhp = jnp.where(hb > 0, dh, jnp.where(hb < 0, 0.5 * dh, 0.0))
            dhp_v[rows, cs] = dhp.astype(BF16)
        return carry

    lax.fori_loop(0, NT, ly, 0)

    finalize()

    C2 = 512

    def dw2_body(c, carry):
        rr = pl.ds(pl.multiple_of(c * C2, C2), C2)
        w2_v[rr, :] = _dot(hT_v[rr, :], df_v[...]).astype(BF16)
        pltpu.make_async_copy(w2_v.at[rr, :], dw2_hbm.at[rr, :], out_sems.at[16 + c]).start()
        return carry

    lax.fori_loop(0, F // C2, dw2_body, 0)

    def dwo_body(c, carry):
        rr = pl.ds(pl.multiple_of(c * C2, C2), C2)
        wo_v[rr, :] = _dot(oT_v[rr, :], ds_v[...]).astype(BF16)
        pltpu.make_async_copy(wo_v.at[rr, :], dwo_hbm.at[rr, :], out_sems.at[24 + c]).start()
        return carry

    lax.fori_loop(0, D // C2, dwo_body, 0)

    dxs_v = gate_v

    def ln_bwd(t, dxnT):
        rows = pl.ds(pl.multiple_of(t * T, T), T)
        xnT = xnT_v[:, rows].astype(F32)
        m1 = jnp.mean(dxnT, axis=0, keepdims=True)
        m2 = jnp.mean(dxnT * xnT, axis=0, keepdims=True)
        u = dxnT - m1 - xnT * m2
        dx = dy_v[rows, :].astype(F32) + jnp.tile(rstd_v[rows, :], (1, D // 128)) * u.T
        dxs_v[rows, :] = dx.astype(BF16)

    dxn_v[...] = jnp.zeros(dxn_v.shape, F32)

    def p3(t, carry):
        rows = pl.ds(pl.multiple_of(t * T, T), T)
        never = jnp.tile((lax.broadcasted_iota(jnp.int32, (8, 128), 0) + t) < 0, (1, T // 128))
        prev = dxn_v[...]
        bq = _dot(wall_v[:, 0:D], phiq_v[:, 0:64, rows].reshape(D, T))
        prev = jnp.where(never[None], bq.reshape(D // 8, 8, T), prev.reshape(D // 8, 8, T)).reshape(D, T)
        ln_bwd(jnp.maximum(t - 1, 0), prev)
        dhp_t = dhp_v[rows, :]
        dpk = []
        dv = []
        bigs = []
        for c in range(8):
            for p in (2 * c, 2 * c + 1):
                phk = phik_v[p, :, rows]
                rhs = jnp.concatenate([vT_v[p * 64:(p + 1) * 64, rows], ones_rows, zrows], axis=0)
                dphi = _dot(at_v[p], rhs)
                dpk.append(_softmax_pm_bwd(phk.astype(F32), dphi).astype(BF16))
                dv.append(_dot(abf_v[p, 0:64, :], phk).astype(BF16))
            bigs.append(_dot(w1_v[c * 128:(c + 1) * 128, :], dhp_t, _NTD))
        big = jnp.concatenate(bigs, axis=0)
        dpkT = jnp.concatenate(dpk, axis=0)
        dvT = jnp.concatenate(dv, axis=0)
        phik_v[:, 0:64, rows] = dpkT.reshape(NP, 64, T)
        vT_v[:, rows] = dvT
        dxn_v[...] = big + bq + _dot(wall_v[:, 2 * D:3 * D], dvT) + _dot(wall_v[:, D:2 * D], dpkT)

        @pl.when(t > 0)
        def _():
            rp = pl.ds(pl.multiple_of((t - 1) * T, T), T)
            pltpu.make_async_copy(dxs_v.at[rp, :], dx_hbm.at[rp, :], out_sems.at[8 + t - 1]).start()

        return carry

    lax.fori_loop(0, NT, p3, 0)
    ln_bwd(NT - 1, dxn_v[...])
    rl = pl.ds((NT - 1) * T, T)
    pltpu.make_async_copy(dxs_v.at[rl, :], dx_hbm.at[rl, :], out_sems.at[8 + NT - 1]).start()

    C1 = 256

    def dw1_body(c, carry):
        rr = pl.ds(pl.multiple_of(c * C1, C1), C1)
        w1_v[rr, :] = _dot(xnT_v[rr, :], dhp_v[...]).astype(BF16)
        pltpu.make_async_copy(w1_v.at[rr, :], dw1_hbm.at[rr, :], out_sems.at[26 + c]).start()
        return carry

    lax.fori_loop(0, D // C1, dw1_body, 0)

    cp_wq.wait()
    cp_wk.wait()
    m_v[...] = jnp.zeros(m_v.shape, F32)

    def g_body(c, carry):
        rr = pl.ds(pl.multiple_of(c * C1, C1), C1)
        rk = pl.ds(pl.multiple_of(D + c * C1, C1), C1)
        xr = xnT_v[rr, :]
        gq = _dot(xr, phiq_v[:, 0:64, :].reshape(D, S), _NTD).astype(BF16)
        gk = _dot(xr, phik_v[:, 0:64, :].reshape(D, S), _NTD).astype(BF16)
        wqk = jnp.concatenate([wt_v[rr, :], wt_v[rk, :]], axis=0)
        for g in range(8):
            cg = slice(g * 128, (g + 1) * 128)
            wb = wbd_v[cg, :]
            wall_v[rr, cg] = _dot(gq[:, cg], wb, _NTD).astype(BF16)
            wall_v[rr, D + g * 128:D + (g + 1) * 128] = _dot(gk[:, cg], wb, _NTD).astype(BF16)
            m_v[g] += _dot(wqk[:, cg], jnp.concatenate([gq[:, cg], gk[:, cg]], axis=0), _TN)
        pltpu.make_async_copy(wall_v.at[rr, 0:2 * D], dwqkv_hbm.at[rr, 0:2 * D], out_sems.at[30 + c]).start()
        wall_v[rr, 2 * D:3 * D] = _dot(xr, vT_v[...], _NTD).astype(BF16)
        pltpu.make_async_copy(wall_v.at[rr, 2 * D:3 * D], dwqkv_hbm.at[rr, 2 * D:3 * D], out_sems.at[34 + c]).start()
        return carry

    lax.fori_loop(0, D // C1, g_body, 0)

    m_r = lax.broadcasted_iota(jnp.int32, (128, 128), 0)
    m_c = lax.broadcasted_iota(jnp.int32, (128, 128), 1)
    bmask = (m_r // 32) == (m_c // 64) * 2 + m_c % 2
    for g in range(8):
        mb = jnp.where(bmask, m_v[g], 0.0).astype(BF16)
        dwphi_ref[g * 128:(g + 1) * 128, :] = _dot(mb, expand, _NTD).astype(BF16)

    for t in range(NT):
        rows = pl.ds(t * T, T)
        pltpu.make_async_copy(x_v.at[rows, :], out_hbm.at[rows, :], out_sems.at[t]).wait()
        pltpu.make_async_copy(dxs_v.at[rows, :], dx_hbm.at[rows, :], out_sems.at[8 + t]).wait()
    for c in range(F // C2):
        rr = pl.ds(c * C2, C2)
        pltpu.make_async_copy(w2_v.at[rr, :], dw2_hbm.at[rr, :], out_sems.at[16 + c]).wait()
    for c in range(D // C2):
        rr = pl.ds(c * C2, C2)
        pltpu.make_async_copy(wo_v.at[rr, :], dwo_hbm.at[rr, :], out_sems.at[24 + c]).wait()
    for c in range(D // C1):
        rr = pl.ds(c * C1, C1)
        pltpu.make_async_copy(w1_v.at[rr, :], dw1_hbm.at[rr, :], out_sems.at[26 + c]).wait()
        pltpu.make_async_copy(wall_v.at[rr, 0:2 * D], dwqkv_hbm.at[rr, 0:2 * D], out_sems.at[30 + c]).wait()
        pltpu.make_async_copy(wall_v.at[rr, 2 * D:3 * D], dwqkv_hbm.at[rr, 2 * D:3 * D], out_sems.at[34 + c]).wait()


@jax.jit
def pallas_recurrent_scan__linear_kernel_hedgehog__dense_activation_relu__prompt_kernel(
    A_x: jax.Array,
    A_wqkv: jax.Array,
    A_w_phi: jax.Array,
    A_wo: jax.Array,
    B_x: jax.Array,
    B_w1: jax.Array,
    B_w2: jax.Array,
    grad_out: jax.Array,
):
    del B_x
    x = A_x.reshape(S, D)
    dy = grad_out.reshape(S, D)
    wphi = A_w_phi.reshape(H * DH, DH)
    any_spec = pl.BlockSpec(memory_space=pl.ANY)
    vmem_spec = pl.BlockSpec(memory_space=pltpu.VMEM)
    out_shape = (
        jax.ShapeDtypeStruct((S, D), BF16),
        jax.ShapeDtypeStruct((S, D), BF16),
        jax.ShapeDtypeStruct((D, 3 * D), BF16),
        jax.ShapeDtypeStruct((H * DH, DH), BF16),
        jax.ShapeDtypeStruct((D, D), BF16),
        jax.ShapeDtypeStruct((D, F), BF16),
        jax.ShapeDtypeStruct((F, D), BF16),
    )
    scratch = [
        pltpu.VMEM((S, D), BF16),
        pltpu.VMEM((S, D), BF16),
        pltpu.VMEM((D, 3 * D), BF16),
        pltpu.VMEM((3 * D, D), BF16),
        pltpu.VMEM((D, D), BF16),
        pltpu.VMEM((D, F), BF16),
        pltpu.VMEM((F, D), BF16),
        pltpu.VMEM((D, 128), BF16),
        pltpu.VMEM((D, S), BF16),
        pltpu.VMEM((S, 128), F32),
        pltpu.VMEM((NP, 128, S), BF16),
        pltpu.VMEM((NP, 128, S), BF16),
        pltpu.VMEM((D, S), BF16),
        pltpu.VMEM((F, S), BF16),
        pltpu.VMEM((S, F), BF16),
        pltpu.VMEM((S, D), BF16),
        pltpu.VMEM((D, S), BF16),
        pltpu.VMEM((S, D), BF16),
        pltpu.VMEM((S, D), BF16),
        pltpu.VMEM((NP, AR, 128), F32),
        pltpu.VMEM((NP, AR, 128), BF16),
        pltpu.VMEM((NP, 128, 128), BF16),
        pltpu.VMEM((8, 128, 128), F32),
        pltpu.VMEM((D, T), F32),
        pltpu.SemaphoreType.DMA((9,)),
        pltpu.SemaphoreType.DMA((NT,)),
        pltpu.SemaphoreType.DMA((8,)),
        pltpu.SemaphoreType.DMA((38,)),
    ]
    outs = pl.pallas_call(
        _kernel,
        out_shape=out_shape,
        in_specs=[any_spec, any_spec, vmem_spec, any_spec, any_spec, any_spec, any_spec],
        out_specs=(any_spec, any_spec, any_spec, vmem_spec, any_spec, any_spec, any_spec),
        scratch_shapes=scratch,
        compiler_params=pltpu.CompilerParams(vmem_limit_bytes=124 * 1024 * 1024),
    )(x, A_wqkv, wphi, A_wo, B_w1, B_w2, dy)
    out, dx, dwqkv, dwphi, dwo, dw1, dw2 = outs
    return (out.reshape(1, S, D), dx.reshape(1, S, D), dwqkv, dwphi.reshape(H, DH, DH), dwo, dw1, dw2)
```

```python
import jax
import jax.numpy as jnp
from jax import lax
import jax.experimental.pallas as pl
import jax.experimental.pallas.tpu as pltpu

S, D, H, DH, F = 2048, 1024, 32, 32, 3584
T = 256
NT = S // T
NP = 16
AR = 80
F32 = jnp.float32
BF16 = jnp.bfloat16

_NN = (((1,), (0,)), ((), ()))
_NTD = (((1,), (1,)), ((), ()))
_TN = (((0,), (0,)), ((), ()))


def _dot(a, b, dims=_NN):
    return lax.dot_general(a, b, dims, preferred_element_type=F32)


def _fold(x, op, axis):
    x = op(x, pltpu.roll(x, 4, axis))
    return op(x, pltpu.roll(x, 2, axis))


def _softmax_pm(pT):
    n = pT.shape[0] // 64
    p4 = pT.reshape(n, 8, 8, T)
    mx = _fold(jnp.max(p4, axis=1), jnp.maximum, 1)
    mn = _fold(jnp.min(p4, axis=1), jnp.minimum, 1)
    ep = jnp.exp(p4 - mx[:, None])
    em = jnp.exp(mn[:, None] - p4)
    sp = _fold(jnp.sum(ep, axis=1), jnp.add, 1)
    sm = _fold(jnp.sum(em, axis=1), jnp.add, 1)
    ap = ep * (1.0 / sp)[:, None]
    am = em * (1.0 / sm)[:, None]
    return ap.reshape(n, 64, T).astype(BF16), am.reshape(n, 64, T).astype(BF16)


def _never(i):
    return jnp.tile((lax.broadcasted_iota(jnp.int32, (8, 128), 0) + i) < 0, (1, T // 128))


def _tie(never, z, x):
    n = x.shape[0]
    return jnp.where(never[None], z.reshape(n // 8, 8, T), x.reshape(n // 8, 8, T)).reshape(n, T)


def _softmax_pm_bwd(a, da):
    a4 = a.reshape(2, 8, 8, T)
    da4 = da.reshape(2, 8, 8, T)
    c = _fold(jnp.sum(a4 * da4, axis=1), jnp.add, 1)
    r = a4 * (da4 - c[:, None])
    return (r[0] - r[1]).reshape(64, T)


def _pair_mask():
    row = lax.broadcasted_iota(jnp.int32, (AR, 128), 0)
    col = lax.broadcasted_iota(jnp.int32, (AR, 128), 1)
    rh = jnp.where(row < 64, row // 32, (row - 64) // 8)
    return rh == (col % 2)


def _kernel(x_hbm, wqkv_hbm, wphi_hbm, wo_hbm, w1_hbm, w2_hbm, dy_hbm,
            out_hbm, dx_hbm, dwqkv_hbm, dwphi_ref, dwo_hbm, dw1_hbm, dw2_hbm,
            x_v, dy_v, wall_v, wt_v, wo_v, w1_v, w2_v, wbd_v,
            xnT_v, rstd_v, phik_v, phiq_v, vT_v, hT_v, dhp_v, df_v, oT_v, ds_v, gate_v,
            acc_v, abf_v, at_v, m_v, dxn_v, st_v, p_v, wphi_ref,
            in_sems, x_sems, w_sems, out_sems):
    def x_copy(t):
        rows = pl.ds(pl.multiple_of(t * T, T), T)
        return pltpu.make_async_copy(x_hbm.at[rows, :], x_v.at[rows, :], x_sems.at[t])

    def w_copy(j):
        r = pl.ds(pl.multiple_of(j * 128, 128), 128)
        return pltpu.make_async_copy(wqkv_hbm.at[r, :], wall_v.at[r, :], w_sems.at[j])

    cp_w1 = pltpu.make_async_copy(w1_hbm, w1_v, in_sems.at[3])
    cp_w2 = pltpu.make_async_copy(w2_hbm, w2_v, in_sems.at[4])
    cp_wo = pltpu.make_async_copy(wo_hbm, wo_v, in_sems.at[5])
    cp_dy = pltpu.make_async_copy(dy_hbm, dy_v, in_sems.at[6])
    cp_wphi = pltpu.make_async_copy(wphi_hbm, wphi_ref, in_sems.at[0])
    cp_wphi.start()
    x_copy(0).start()
    w_copy(0).start()
    w_copy(1).start()

    def layernorm(t, pace=None):
        rows = pl.ds(pl.multiple_of(t * T, T), T)
        x = x_v[rows, :].astype(F32)
        if pace is not None:
            x = pace(x)
        mu = jnp.mean(x, axis=1, keepdims=True)
        xc = x - mu
        var = jnp.mean(xc * xc, axis=1, keepdims=True)
        rstd = lax.rsqrt(var + 1e-5)
        rstd_v[rows, :] = jnp.broadcast_to(rstd, (T, 128))
        xn = (xc * rstd).astype(BF16)
        gate_v[rows, :] = xn
        xnT_v[:, rows] = xn.T

    def zero_body(i, carry):
        acc_v[i] = jnp.zeros((AR, 128), F32)
        return carry

    lax.fori_loop(0, NP, zero_body, 0)

    x_copy(0).wait()
    w_copy(2).start()
    w_copy(3).start()
    x_copy(1).start()
    layernorm(0)
    cp_wphi.wait()
    e_r = lax.broadcasted_iota(jnp.int32, (DH, 128), 0)
    e_c = lax.broadcasted_iota(jnp.int32, (DH, 128), 1)
    expand = jnp.where((e_c % 64) // 2 == e_r, 1.0, 0.0).astype(BF16)
    m_r = lax.broadcasted_iota(jnp.int32, (128, 128), 0)
    m_c = lax.broadcasted_iota(jnp.int32, (128, 128), 1)
    bmask = (m_r // 32) == (m_c // 64) * 2 + m_c % 2
    wexp = _dot(wphi_ref[...], expand).reshape(8, 128, 128)
    wbd_v[...] = jnp.where(bmask[None], wexp, 0.0).reshape(D, 128).astype(BF16)

    for i in range(4):
        w_copy(2 * i).wait()
        w_copy(2 * i + 1).wait()
        if i < 2:
            w_copy(2 * i + 4).start()
            w_copy(2 * i + 5).start()
        if i >= 1:
            x_copy(i + 1).start()
        if i == 2:
            x_copy(1).wait()
            layernorm(1)
        r = slice(i * 256, (i + 1) * 256)
        w_in = wall_v[r, :]
        w = jnp.concatenate(
            [_dot(w_in[:, j * 128:(j + 1) * 128], wbd_v[(j % 8) * 128:(j % 8 + 1) * 128, :]).astype(BF16)
             for j in range(16)] + [w_in[:, 2 * D:3 * D]], axis=1)
        wall_v[r, :] = w
        wT = w.T
        wt_v[:, r] = wT
        part = _dot(wT, xnT_v[r, 0:T])
        if i == 0:
            p_v[...] = part
        else:
            p_v[...] += part
    for t in range(5, NT):
        x_copy(t).start()
    cp_w1.start()
    cp_w2.start()
    cp_dy.start()
    cp_wo.start()

    ones_rows = jnp.ones((AR - 64, T), BF16)

    def l1(t, carry):
        @pl.when(t + 2 < NT)
        def _():
            x_copy(t + 2).wait()

        rows = pl.ds(pl.multiple_of(t * T, T), T)
        never = _never(t)
        xnT = xnT_v[:, pl.ds(pl.multiple_of((t + 1) * T, T), T)]
        HD = D // 2
        vT = p_v[2 * D:3 * D, :].astype(BF16)
        vT_v[:, rows] = vT
        old = [p_v[c * HD:(c + 1) * HD, :] for c in range(4)]
        order = [4, 5, 2, 3, 0, 1]
        new = {}

        def mm(c):
            new[c] = _dot(wt_v[c * HD:(c + 1) * HD, :], xnT)

        def feat(dst, c, z):
            ap, am = _softmax_pm(_tie(never, z, old[c]))
            pr = slice((c % 2) * 8, (c % 2) * 8 + 8)
            dst[pr, 0:64, rows] = ap
            dst[pr, 64:128, rows] = am
            return ap, am

        def a_acc(p0, kp, km):
            for u in range(8):
                p = p0 + u
                lhs = jnp.concatenate([vT[p * 64:(p + 1) * 64], ones_rows], axis=0)
                rhs = jnp.concatenate([kp[u], km[u]], axis=0)
                acc_v[p] += _dot(lhs, rhs, _NTD)

        mm(4)
        k0 = feat(phik_v, 2, new[4])
        mm(5)
        k1 = feat(phik_v, 3, new[5])
        mm(2)
        a_acc(0, *k0)

        def pace(x):
            v4 = jnp.concatenate([new[2], new[2]], axis=0).reshape(T // 8, 4, 8, T)
            z = jnp.concatenate([v4[:, q] for q in range(4)], axis=2)
            m = jnp.tile(never, (1, D // T))[None]
            return jnp.where(m, z, x.reshape(T // 8, 8, D)).reshape(T, D)

        layernorm(jnp.minimum(t + 2, NT - 1), pace)
        mm(3)
        a_acc(8, *k1)
        feat(phiq_v, 0, new[3])
        mm(0)
        feat(phiq_v, 1, new[0])
        mm(1)
        for c in order:
            p_v[c * HD:(c + 1) * HD, :] = new[c]
        return carry

    lax.fori_loop(0, NT - 1, l1, 0)

    cp_wq = pltpu.make_async_copy(wqkv_hbm.at[:, 0:D], wt_v.at[0:D, :], in_sems.at[7])
    cp_wk = pltpu.make_async_copy(wqkv_hbm.at[:, D:2 * D], wt_v.at[D:2 * D, :], in_sems.at[8])
    cp_wq.start()
    cp_wk.start()

    zpad = jnp.zeros((128 - AR, 128), F32)

    def finalize_pair(p):
        a = jnp.where(_pair_mask(), acc_v[p], 0.0)
        abf_v[p] = a.astype(BF16)
        at_v[p] = jnp.concatenate([a, zpad], axis=0).T.astype(BF16)

    cp_w1.wait()
    cp_w2.wait()
    cp_dy.wait()

    def lx(t, carry):
        rows = pl.ds(pl.multiple_of(t * T, T), T)
        pre = _dot(gate_v[rows, :], w1_v[...])
        never = _never(t)
        rl = pl.ds((NT - 1) * T, T)
        r2 = pl.multiple_of(t * 128, 128)
        two = pl.ds(pl.multiple_of(2 * t, 2), 2)
        kp, km = _softmax_pm(_tie(never, pre[0:128, 0:T], p_v[pl.ds(D + r2, 128), :]))
        qp, qm = _softmax_pm(_tie(never, pre[128:256, 0:T], p_v[pl.ds(r2, 128), :]))
        vT = p_v[pl.ds(2 * D + r2, 128), :].astype(BF16)
        phik_v[two, 0:64, rl] = kp
        phik_v[two, 64:128, rl] = km
        phiq_v[two, 0:64, rl] = qp
        phiq_v[two, 64:128, rl] = qm
        vT_v[pl.ds(r2, 128), rl] = vT
        for u in range(2):
            lhs = jnp.concatenate([vT[u * 64:(u + 1) * 64], ones_rows], axis=0)
            rhs = jnp.concatenate([kp[u], km[u]], axis=0)
            acc_v[2 * t + u] += _dot(lhs, rhs, _NTD)
            finalize_pair(2 * t + u)
            acc_v[2 * t + u] = jnp.zeros((AR, 128), F32)
        h = jnp.where(pre == 0.0, -0.0, jnp.maximum(pre, 0.0)).astype(BF16)
        dhp_v[rows, :] = h
        hT_v[:, rows] = h.T
        f = _dot(h, w2_v[...])
        sig = 0.5 * jnp.tanh(0.5 * f) + 0.5
        gate = f * sig
        dy = dy_v[rows, :].astype(F32)
        gate_v[rows, :] = gate.astype(BF16)
        ds_v[rows, :] = (dy * gate).astype(BF16)
        df_v[rows, :] = (dy * (sig * (1.0 + f * (1.0 - sig)))).astype(BF16)
        return carry

    lax.fori_loop(0, NT, lx, 0)

    cp_wo.wait()
    zrows = jnp.zeros((128 - AR, T), BF16)

    def ly(t, carry):
        rows = pl.ds(pl.multiple_of(t * T, T), T)
        ds = ds_v[rows, :]
        phiq = [phiq_v[p, :, rows] for p in range(NP)]
        do4, o4, rd = [], [], []
        for c in range(8):
            for p in (2 * c, 2 * c + 1):
                n = _dot(abf_v[p], phiq[p])
                r = 1.0 / (n[64:AR].reshape(2, 8, T) + 1e-6)
                rd.append(r)
                o4.append(n[0:64].reshape(2, 4, 8, T) * r[:, None])
            d = _dot(wo_v[c * 128:(c + 1) * 128, :], ds, _NTD).reshape(2, 2, 4, 8, T)
            do4 += [d[0], d[1]]
        oTb = jnp.concatenate([o.reshape(64, T).astype(BF16) for o in o4], axis=0)
        oT_v[:, rows] = oTb
        o_n = oTb.T

        def attn_bwd(p):
            dn = (do4[p] * rd[p][:, None]).reshape(64, T).astype(BF16)
            tt = jnp.sum(do4[p] * o4[p], axis=1)
            tt = tt + pltpu.roll(tt, 4, 1)
            tt = tt + pltpu.roll(tt, 2, 1)
            tt = tt + pltpu.roll(tt, 1, 1)
            dd = (tt * rd[p] * (-0.125)).reshape(16, T).astype(BF16)
            lhs = jnp.concatenate([dn, dd], axis=0)
            dphi = _dot(at_v[p], jnp.concatenate([lhs, zrows], axis=0))
            dp = _softmax_pm_bwd(phiq[p].astype(F32), dphi)
            acc_v[p] += _dot(lhs, phiq[p], _NTD)
            phiq_v[p, 0:64, rows] = dp.astype(BF16)

        dfs = []
        for c in range(4):
            attn_bwd(c)
            cs = slice(c * 256, (c + 1) * 256)
            s = _dot(o_n, wo_v[:, cs])
            x_v[rows, cs] = (x_v[rows, cs].astype(F32) + s * gate_v[rows, cs].astype(F32)).astype(BF16)
            dfs.append((df_v[rows, cs].astype(F32) * s).astype(BF16))
        df = jnp.concatenate(dfs, axis=1)
        df_v[rows, :] = df
        pltpu.make_async_copy(x_v.at[rows, :], out_hbm.at[rows, :], out_sems.at[t]).start()

        for c in range(14):
            if c < 12:
                attn_bwd(4 + c)
            cs = slice(c * 256, (c + 1) * 256)
            dh = _dot(df, w2_v[cs, :], _NTD)
            hb = lax.bitcast_convert_type(dhp_v[rows, cs].astype(F32), jnp.int32)
            dhp = jnp.where(hb > 0, dh, jnp.where(hb < 0, 0.5 * dh, 0.0))
            dhp_v[rows, cs] = dhp.astype(BF16)
        return carry

    lax.fori_loop(0, NT, ly, 0)

    C2 = 512

    def dw2_body(c, carry):
        rr = pl.ds(pl.multiple_of(c * C2, C2), C2)
        for u in range(3):
            finalize_pair(jnp.minimum(3 * c + u, NP - 1))
        w2_v[rr, :] = _dot(hT_v[rr, :], df_v[...]).astype(BF16)
        pltpu.make_async_copy(w2_v.at[rr, :], dw2_hbm.at[rr, :], out_sems.at[16 + c]).start()
        return carry

    lax.fori_loop(0, F // C2, dw2_body, 0)

    def dwo_body(c, carry):
        rr = pl.ds(pl.multiple_of(c * C2, C2), C2)
        wo_v[rr, :] = _dot(oT_v[rr, :], ds_v[...]).astype(BF16)
        pltpu.make_async_copy(wo_v.at[rr, :], dwo_hbm.at[rr, :], out_sems.at[24 + c]).start()
        return carry

    lax.fori_loop(0, D // C2, dwo_body, 0)

    dxs_v = gate_v

    def ln_stats(dxnT, xnT):
        m1 = jnp.mean(dxnT, axis=0, keepdims=True)
        m2 = jnp.mean(dxnT * xnT, axis=0, keepdims=True)
        return m1, m2

    def ln_bwd_chunk(rows, cols, n, dxnT, m1, m2):
        u = dxnT - m1 - xnT_v[cols, rows].astype(F32) * m2
        dx = dy_v[rows, cols].astype(F32) + jnp.tile(rstd_v[rows, :], (1, n // 128)) * u.T
        dxs_v[rows, cols] = dx.astype(BF16)

    dxn_v[...] = jnp.zeros(dxn_v.shape, F32)

    def p3(t, carry):
        rows = pl.ds(pl.multiple_of(t * T, T), T)
        rp = pl.ds(pl.multiple_of(jnp.maximum(t - 1, 0) * T, T), T)
        never = _never(t)
        prev = dxn_v[...]
        bq = _dot(wall_v[:, 0:D], phiq_v[:, 0:64, rows].reshape(D, T))
        m1, m2 = ln_stats(_tie(never, bq, prev), xnT_v[:, rp].astype(F32))
        dhp_t = dhp_v[rows, :]
        dpk = []
        dv = []
        bigs = []
        for c in range(8):
            for p in (2 * c, 2 * c + 1):
                phk = phik_v[p, :, rows]
                rhs = jnp.concatenate([vT_v[p * 64:(p + 1) * 64, rows], ones_rows, zrows], axis=0)
                dphi = _dot(at_v[p], rhs)
                dpk.append(_softmax_pm_bwd(phk.astype(F32), dphi).astype(BF16))
                dv.append(_dot(abf_v[p, 0:64, :], phk).astype(BF16))
            cs = slice(c * 128, (c + 1) * 128)
            bigs.append(_dot(w1_v[cs, :], dhp_t, _NTD))
            ln_bwd_chunk(rp, cs, 128, _tie(never, bigs[c], prev[cs]), m1, m2)
        big = jnp.concatenate(bigs, axis=0)
        dpkT = jnp.concatenate(dpk, axis=0)
        dvT = jnp.concatenate(dv, axis=0)
        phik_v[:, 0:64, rows] = dpkT.reshape(NP, 64, T)
        vT_v[:, rows] = dvT
        dxn_v[...] = big + bq + _dot(wall_v[:, 2 * D:3 * D], dvT) + _dot(wall_v[:, D:2 * D], dpkT)

        @pl.when(t > 0)
        def _():
            pltpu.make_async_copy(dxs_v.at[rp, :], dx_hbm.at[rp, :], out_sems.at[8 + t - 1]).start()

        return carry

    lax.fori_loop(0, NT, p3, 0)
    rl = pl.ds((NT - 1) * T, T)
    m1l, m2l = ln_stats(dxn_v[...], xnT_v[:, rl].astype(F32))
    st_v[0:8, :] = jnp.broadcast_to(m1l, (8, T))
    st_v[8:16, :] = jnp.broadcast_to(m2l, (8, T))

    C1 = 256

    def dw1_body(c, carry):
        rr = pl.ds(pl.multiple_of(c * C1, C1), C1)
        never = _never(c)
        res = _dot(xnT_v[rr, :], dhp_v[...])
        ln_bwd_chunk(rl, rr, C1, _tie(never, res[:, 0:T], dxn_v[rr, :]), st_v[0:1, :], st_v[8:9, :])
        w1_v[rr, :] = res.astype(BF16)
        pltpu.make_async_copy(w1_v.at[rr, :], dw1_hbm.at[rr, :], out_sems.at[26 + c]).start()
        return carry

    lax.fori_loop(0, D // C1, dw1_body, 0)
    pltpu.make_async_copy(dxs_v.at[rl, :], dx_hbm.at[rl, :], out_sems.at[8 + NT - 1]).start()

    cp_wq.wait()
    cp_wk.wait()
    m_v[...] = jnp.zeros(m_v.shape, F32)

    CG = 128

    def g_body(c, carry):
        rr = pl.ds(pl.multiple_of(c * CG, CG), CG)
        rk = pl.ds(pl.multiple_of(D + c * CG, CG), CG)
        xr = xnT_v[rr, :]
        gq = _dot(xr, phiq_v[:, 0:64, :].reshape(D, S), _NTD).astype(BF16)
        gk = _dot(xr, phik_v[:, 0:64, :].reshape(D, S), _NTD).astype(BF16)
        wqk = jnp.concatenate([wt_v[rr, :], wt_v[rk, :]], axis=0)
        for g in range(8):
            cg = slice(g * 128, (g + 1) * 128)
            wb = wbd_v[cg, :]
            wall_v[rr, cg] = _dot(gq[:, cg], wb, _NTD).astype(BF16)
            wall_v[rr, D + g * 128:D + (g + 1) * 128] = _dot(gk[:, cg], wb, _NTD).astype(BF16)
            m_v[g] += _dot(wqk[:, cg], jnp.concatenate([gq[:, cg], gk[:, cg]], axis=0), _TN)
        pltpu.make_async_copy(wall_v.at[rr, 0:2 * D], dwqkv_hbm.at[rr, 0:2 * D], out_sems.at[30 + c]).start()
        wall_v[rr, 2 * D:3 * D] = _dot(xr, vT_v[...], _NTD).astype(BF16)
        pltpu.make_async_copy(wall_v.at[rr, 2 * D:3 * D], dwqkv_hbm.at[rr, 2 * D:3 * D], out_sems.at[38 + c]).start()
        return carry

    lax.fori_loop(0, D // CG, g_body, 0)

    for g in range(8):
        mb = jnp.where(bmask, m_v[g], 0.0).astype(BF16)
        dwphi_ref[g * 128:(g + 1) * 128, :] = _dot(mb, expand, _NTD).astype(BF16)

    for t in range(NT):
        rows = pl.ds(t * T, T)
        pltpu.make_async_copy(x_v.at[rows, :], out_hbm.at[rows, :], out_sems.at[t]).wait()
        pltpu.make_async_copy(dxs_v.at[rows, :], dx_hbm.at[rows, :], out_sems.at[8 + t]).wait()
    for c in range(F // C2):
        rr = pl.ds(c * C2, C2)
        pltpu.make_async_copy(w2_v.at[rr, :], dw2_hbm.at[rr, :], out_sems.at[16 + c]).wait()
    for c in range(D // C2):
        rr = pl.ds(c * C2, C2)
        pltpu.make_async_copy(wo_v.at[rr, :], dwo_hbm.at[rr, :], out_sems.at[24 + c]).wait()
    for c in range(D // C1):
        rr = pl.ds(c * C1, C1)
        pltpu.make_async_copy(w1_v.at[rr, :], dw1_hbm.at[rr, :], out_sems.at[26 + c]).wait()
    for c in range(D // CG):
        rr = pl.ds(c * CG, CG)
        pltpu.make_async_copy(wall_v.at[rr, 0:2 * D], dwqkv_hbm.at[rr, 0:2 * D], out_sems.at[30 + c]).wait()
        pltpu.make_async_copy(wall_v.at[rr, 2 * D:3 * D], dwqkv_hbm.at[rr, 2 * D:3 * D], out_sems.at[38 + c]).wait()


@jax.jit
def pallas_recurrent_scan__linear_kernel_hedgehog__dense_activation_relu__prompt_kernel(
    A_x: jax.Array,
    A_wqkv: jax.Array,
    A_w_phi: jax.Array,
    A_wo: jax.Array,
    B_x: jax.Array,
    B_w1: jax.Array,
    B_w2: jax.Array,
    grad_out: jax.Array,
):
    del B_x
    x = A_x.reshape(S, D)
    dy = grad_out.reshape(S, D)
    wphi = A_w_phi.reshape(H * DH, DH)
    any_spec = pl.BlockSpec(memory_space=pl.ANY)
    vmem_spec = pl.BlockSpec(memory_space=pltpu.VMEM)
    out_shape = (
        jax.ShapeDtypeStruct((S, D), BF16),
        jax.ShapeDtypeStruct((S, D), BF16),
        jax.ShapeDtypeStruct((D, 3 * D), BF16),
        jax.ShapeDtypeStruct((H * DH, DH), BF16),
        jax.ShapeDtypeStruct((D, D), BF16),
        jax.ShapeDtypeStruct((D, F), BF16),
        jax.ShapeDtypeStruct((F, D), BF16),
    )
    scratch = [
        pltpu.VMEM((S, D), BF16),
        pltpu.VMEM((S, D), BF16),
        pltpu.VMEM((D, 3 * D), BF16),
        pltpu.VMEM((3 * D, D), BF16),
        pltpu.VMEM((D, D), BF16),
        pltpu.VMEM((D, F), BF16),
        pltpu.VMEM((F, D), BF16),
        pltpu.VMEM((D, 128), BF16),
        pltpu.VMEM((D, S), BF16),
        pltpu.VMEM((S, 128), F32),
        pltpu.VMEM((NP, 128, S), BF16),
        pltpu.VMEM((NP, 128, S), BF16),
        pltpu.VMEM((D, S), BF16),
        pltpu.VMEM((F, S), BF16),
        pltpu.VMEM((S, F), BF16),
        pltpu.VMEM((S, D), BF16),
        pltpu.VMEM((D, S), BF16),
        pltpu.VMEM((S, D), BF16),
        pltpu.VMEM((S, D), BF16),
        pltpu.VMEM((NP, AR, 128), F32),
        pltpu.VMEM((NP, AR, 128), BF16),
        pltpu.VMEM((NP, 128, 128), BF16),
        pltpu.VMEM((8, 128, 128), F32),
        pltpu.VMEM((D, T), F32),
        pltpu.VMEM((16, T), F32),
        pltpu.VMEM((3 * D, T), F32),
        pltpu.VMEM((H * DH, DH), BF16),
        pltpu.SemaphoreType.DMA((9,)),
        pltpu.SemaphoreType.DMA((NT,)),
        pltpu.SemaphoreType.DMA((8,)),
        pltpu.SemaphoreType.DMA((46,)),
    ]
    outs = pl.pallas_call(
        _kernel,
        out_shape=out_shape,
        in_specs=[any_spec] * 7,
        out_specs=(any_spec, any_spec, any_spec, vmem_spec, any_spec, any_spec, any_spec),
        scratch_shapes=scratch,
        compiler_params=pltpu.CompilerParams(vmem_limit_bytes=124 * 1024 * 1024),
    )(x, A_wqkv, wphi, A_wo, B_w1, B_w2, dy)
    out, dx, dwqkv, dwphi, dwo, dw1, dw2 = outs
    return (out.reshape(1, S, D), dx.reshape(1, S, D), dwqkv, dwphi.reshape(H, DH, DH), dwo, dw1, dw2)
```

```python
import jax
import jax.numpy as jnp
from jax import lax
import jax.experimental.pallas as pl
import jax.experimental.pallas.tpu as pltpu

S, D, H, DH, F = 2048, 1024, 32, 32, 3584
T = 256
NT = S // T
NP = 16
AR = 80
F32 = jnp.float32
BF16 = jnp.bfloat16

_NN = (((1,), (0,)), ((), ()))
_NTD = (((1,), (1,)), ((), ()))
_TN = (((0,), (0,)), ((), ()))


def _dot(a, b, dims=_NN):
    return lax.dot_general(a, b, dims, preferred_element_type=F32)


def _fold(x, op, axis):
    x = op(x, pltpu.roll(x, 4, axis))
    return op(x, pltpu.roll(x, 2, axis))


def _softmax_pm(pT):
    n = pT.shape[0] // 64
    p4 = pT.reshape(n, 8, 8, T)
    mx = _fold(jnp.max(p4, axis=1), jnp.maximum, 1)
    mn = _fold(jnp.min(p4, axis=1), jnp.minimum, 1)
    ep = jnp.exp(p4 - mx[:, None])
    em = jnp.exp(mn[:, None] - p4)
    sp = _fold(jnp.sum(ep, axis=1), jnp.add, 1)
    sm = _fold(jnp.sum(em, axis=1), jnp.add, 1)
    ap = ep * (1.0 / sp)[:, None]
    am = em * (1.0 / sm)[:, None]
    return ap.reshape(n, 64, T).astype(BF16), am.reshape(n, 64, T).astype(BF16)


def _never(i):
    return jnp.tile((lax.broadcasted_iota(jnp.int32, (8, 128), 0) + i) < 0, (1, T // 128))


def _tie(never, z, x):
    n = x.shape[0]
    return jnp.where(never[None], z.reshape(n // 8, 8, T), x.reshape(n // 8, 8, T)).reshape(n, T)


def _softmax_pm_bwd(a, da):
    a4 = a.reshape(2, 8, 8, T)
    da4 = da.reshape(2, 8, 8, T)
    c = _fold(jnp.sum(a4 * da4, axis=1), jnp.add, 1)
    r = a4 * (da4 - c[:, None])
    return (r[0] - r[1]).reshape(64, T)


def _pair_mask():
    row = lax.broadcasted_iota(jnp.int32, (AR, 128), 0)
    col = lax.broadcasted_iota(jnp.int32, (AR, 128), 1)
    rh = jnp.where(row < 64, row // 32, (row - 64) // 8)
    return rh == (col % 2)


def _kernel(x_hbm, wqkv_hbm, wphi_hbm, wo_hbm, w1_hbm, w2_hbm, dy_hbm,
            out_hbm, dx_hbm, dwqkv_hbm, dwphi_hbm, dwo_hbm, dw1_hbm, dw2_hbm,
            x_v, dy_v, wall_v, wt_v, wo_v, w1_v, w2_v, wbd_v,
            xnT_v, rstd_v, phik_v, phiq_v, vT_v, hT_v, dhp_v, df_v, oT_v, ds_v, gate_v,
            acc_v, abf_v, at_v, m_v, dxn_v, st_v, p_v, wphi_ref,
            in_sems, x_sems, w_sems, out_sems):
    def x_copy(t):
        rows = pl.ds(pl.multiple_of(t * T, T), T)
        return pltpu.make_async_copy(x_hbm.at[rows, :], x_v.at[rows, :], x_sems.at[t])

    def w_copy(j):
        r = pl.ds(pl.multiple_of(j * 128, 128), 128)
        return pltpu.make_async_copy(wqkv_hbm.at[r, :], wall_v.at[r, :], w_sems.at[j])

    cp_w1 = pltpu.make_async_copy(w1_hbm, w1_v, in_sems.at[3])
    cp_w2 = pltpu.make_async_copy(w2_hbm, w2_v, in_sems.at[4])
    cp_wo = pltpu.make_async_copy(wo_hbm, wo_v, in_sems.at[5])
    cp_dy = pltpu.make_async_copy(dy_hbm, dy_v, in_sems.at[6])
    cp_wphi = pltpu.make_async_copy(wphi_hbm, wphi_ref, in_sems.at[0])
    cp_wphi.start()
    x_copy(0).start()
    w_copy(0).start()
    w_copy(1).start()

    def layernorm(t, pace=None):
        rows = pl.ds(pl.multiple_of(t * T, T), T)
        x = x_v[rows, :].astype(F32)
        if pace is not None:
            x = pace(x)
        mu = jnp.mean(x, axis=1, keepdims=True)
        xc = x - mu
        var = jnp.mean(xc * xc, axis=1, keepdims=True)
        rstd = lax.rsqrt(var + 1e-5)
        rstd_v[rows, :] = jnp.broadcast_to(rstd, (T, 128))
        xn = (xc * rstd).astype(BF16)
        gate_v[rows, :] = xn
        xnT_v[:, rows] = xn.T

    def zero_body(i, carry):
        acc_v[i] = jnp.zeros((AR, 128), F32)
        dxn_v[pl.ds(pl.multiple_of(i * 64, 64), 64), :] = jnp.zeros((64, T), F32)
        m_v[i // 2, pl.ds(pl.multiple_of((i % 2) * 64, 64), 64), :] = jnp.zeros((64, 128), F32)
        return carry

    lax.fori_loop(0, NP, zero_body, 0)

    x_copy(0).wait()
    w_copy(2).start()
    w_copy(3).start()
    x_copy(1).start()
    layernorm(0)
    cp_wphi.wait()
    e_r = lax.broadcasted_iota(jnp.int32, (DH, 128), 0)
    e_c = lax.broadcasted_iota(jnp.int32, (DH, 128), 1)
    expand = jnp.where((e_c % 64) // 2 == e_r, 1.0, 0.0).astype(BF16)
    m_r = lax.broadcasted_iota(jnp.int32, (128, 128), 0)
    m_c = lax.broadcasted_iota(jnp.int32, (128, 128), 1)
    bmask = (m_r // 32) == (m_c // 64) * 2 + m_c % 2
    wexp = _dot(wphi_ref[...], expand).reshape(8, 128, 128)
    wbd_v[...] = jnp.where(bmask[None], wexp, 0.0).reshape(D, 128).astype(BF16)

    for i in range(4):
        w_copy(2 * i).wait()
        w_copy(2 * i + 1).wait()
        if i < 2:
            w_copy(2 * i + 4).start()
            w_copy(2 * i + 5).start()
        if i >= 1:
            x_copy(i + 1).start()
        if i == 2:
            x_copy(1).wait()
            layernorm(1)
        r = slice(i * 256, (i + 1) * 256)
        w_in = wall_v[r, :]
        w = jnp.concatenate(
            [_dot(w_in[:, j * 128:(j + 1) * 128], wbd_v[(j % 8) * 128:(j % 8 + 1) * 128, :]).astype(BF16)
             for j in range(16)] + [w_in[:, 2 * D:3 * D]], axis=1)
        wall_v[r, :] = w
        wT = w.T
        wt_v[:, r] = wT
        part = _dot(wT, xnT_v[r, 0:T])
        if i == 0:
            p_v[...] = part
        else:
            p_v[...] += part
    for t in range(5, NT):
        x_copy(t).start()
    cp_w1.start()
    cp_w2.start()
    cp_dy.start()
    cp_wo.start()

    ones_rows = jnp.ones((AR - 64, T), BF16)

    def l1(t, carry):
        @pl.when(t + 2 < NT)
        def _():
            x_copy(t + 2).wait()

        rows = pl.ds(pl.multiple_of(t * T, T), T)
        never = _never(t)
        xnT = xnT_v[:, pl.ds(pl.multiple_of((t + 1) * T, T), T)]
        HD = D // 2
        vT = p_v[2 * D:3 * D, :].astype(BF16)
        vT_v[:, rows] = vT
        old = [p_v[c * HD:(c + 1) * HD, :] for c in range(4)]
        order = [4, 5, 2, 3, 0, 1]
        new = {}

        def mm(c):
            new[c] = _dot(wt_v[c * HD:(c + 1) * HD, :], xnT)

        def feat(dst, c, z):
            ap, am = _softmax_pm(_tie(never, z, old[c]))
            pr = slice((c % 2) * 8, (c % 2) * 8 + 8)
            dst[pr, 0:64, rows] = ap
            dst[pr, 64:128, rows] = am
            return ap, am

        def a_acc(p0, kp, km):
            for u in range(8):
                p = p0 + u
                lhs = jnp.concatenate([vT[p * 64:(p + 1) * 64], ones_rows], axis=0)
                rhs = jnp.concatenate([kp[u], km[u]], axis=0)
                acc_v[p] += _dot(lhs, rhs, _NTD)

        mm(4)
        k0 = feat(phik_v, 2, new[4])
        mm(5)
        k1 = feat(phik_v, 3, new[5])
        mm(2)
        a_acc(0, *k0)

        def pace(x):
            v4 = jnp.concatenate([new[2], new[2]], axis=0).reshape(T // 8, 4, 8, T)
            z = jnp.concatenate([v4[:, q] for q in range(4)], axis=2)
            m = jnp.tile(never, (1, D // T))[None]
            return jnp.where(m, z, x.reshape(T // 8, 8, D)).reshape(T, D)

        layernorm(jnp.minimum(t + 2, NT - 1), pace)
        mm(3)
        a_acc(8, *k1)
        feat(phiq_v, 0, new[3])
        mm(0)
        feat(phiq_v, 1, new[0])
        mm(1)
        for c in order:
            p_v[c * HD:(c + 1) * HD, :] = new[c]
        return carry

    lax.fori_loop(0, NT - 1, l1, 0)

    cp_wq = pltpu.make_async_copy(wqkv_hbm.at[:, 0:D], wt_v.at[0:D, :], in_sems.at[7])
    cp_wk = pltpu.make_async_copy(wqkv_hbm.at[:, D:2 * D], wt_v.at[D:2 * D, :], in_sems.at[8])
    cp_wq.start()
    cp_wk.start()

    zpad = jnp.zeros((128 - AR, 128), F32)

    def finalize_pair(p):
        a = jnp.where(_pair_mask(), acc_v[p], 0.0)
        abf_v[p] = a.astype(BF16)
        at_v[p] = jnp.concatenate([a, zpad], axis=0).T.astype(BF16)

    cp_w1.wait()
    cp_w2.wait()
    cp_dy.wait()

    def lx(t, carry):
        rows = pl.ds(pl.multiple_of(t * T, T), T)
        pre = _dot(gate_v[rows, :], w1_v[...])
        never = _never(t)
        rl = pl.ds((NT - 1) * T, T)
        r2 = pl.multiple_of(t * 128, 128)
        two = pl.ds(pl.multiple_of(2 * t, 2), 2)
        kp, km = _softmax_pm(_tie(never, pre[0:128, 0:T], p_v[pl.ds(D + r2, 128), :]))
        qp, qm = _softmax_pm(_tie(never, pre[128:256, 0:T], p_v[pl.ds(r2, 128), :]))
        vT = p_v[pl.ds(2 * D + r2, 128), :].astype(BF16)
        phik_v[two, 0:64, rl] = kp
        phik_v[two, 64:128, rl] = km
        phiq_v[two, 0:64, rl] = qp
        phiq_v[two, 64:128, rl] = qm
        vT_v[pl.ds(r2, 128), rl] = vT
        for u in range(2):
            lhs = jnp.concatenate([vT[u * 64:(u + 1) * 64], ones_rows], axis=0)
            rhs = jnp.concatenate([kp[u], km[u]], axis=0)
            acc_v[2 * t + u] += _dot(lhs, rhs, _NTD)
            finalize_pair(2 * t + u)
            acc_v[2 * t + u] = jnp.zeros((AR, 128), F32)
        h = jnp.where(pre == 0.0, -0.0, jnp.maximum(pre, 0.0)).astype(BF16)
        dhp_v[rows, :] = h
        hT_v[:, rows] = h.T
        f = _dot(h, w2_v[...])
        sig = 0.5 * jnp.tanh(0.5 * f) + 0.5
        gate = f * sig
        dy = dy_v[rows, :].astype(F32)
        gate_v[rows, :] = gate.astype(BF16)
        ds_v[rows, :] = (dy * gate).astype(BF16)
        df_v[rows, :] = (dy * (sig * (1.0 + f * (1.0 - sig)))).astype(BF16)
        return carry

    lax.fori_loop(0, NT, lx, 0)

    cp_wo.wait()
    zrows = jnp.zeros((128 - AR, T), BF16)

    def ly(t, carry):
        rows = pl.ds(pl.multiple_of(t * T, T), T)
        ds = ds_v[rows, :]
        phiq = [phiq_v[p, :, rows] for p in range(NP)]
        do4, o4, rd = [], [], []
        for c in range(8):
            for p in (2 * c, 2 * c + 1):
                n = _dot(abf_v[p], phiq[p])
                r = 1.0 / (n[64:AR].reshape(2, 8, T) + 1e-6)
                rd.append(r)
                o4.append(n[0:64].reshape(2, 4, 8, T) * r[:, None])
            d = _dot(wo_v[c * 128:(c + 1) * 128, :], ds, _NTD).reshape(2, 2, 4, 8, T)
            do4 += [d[0], d[1]]
        oTb = jnp.concatenate([o.reshape(64, T).astype(BF16) for o in o4], axis=0)
        oT_v[:, rows] = oTb
        o_n = oTb.T

        def attn_bwd(p):
            dn = (do4[p] * rd[p][:, None]).reshape(64, T).astype(BF16)
            tt = jnp.sum(do4[p] * o4[p], axis=1)
            tt = tt + pltpu.roll(tt, 4, 1)
            tt = tt + pltpu.roll(tt, 2, 1)
            tt = tt + pltpu.roll(tt, 1, 1)
            dd = (tt * rd[p] * (-0.125)).reshape(16, T).astype(BF16)
            lhs = jnp.concatenate([dn, dd], axis=0)
            dphi = _dot(at_v[p], jnp.concatenate([lhs, zrows], axis=0))
            dp = _softmax_pm_bwd(phiq[p].astype(F32), dphi)
            acc_v[p] += _dot(lhs, phiq[p], _NTD)
            phiq_v[p, 0:64, rows] = dp.astype(BF16)

        dfs = []
        for c in range(4):
            attn_bwd(c)
            cs = slice(c * 256, (c + 1) * 256)
            s = _dot(o_n, wo_v[:, cs])
            x_v[rows, cs] = (x_v[rows, cs].astype(F32) + s * gate_v[rows, cs].astype(F32)).astype(BF16)
            dfs.append((df_v[rows, cs].astype(F32) * s).astype(BF16))
        df = jnp.concatenate(dfs, axis=1)
        df_v[rows, :] = df
        pltpu.make_async_copy(x_v.at[rows, :], out_hbm.at[rows, :], out_sems.at[t]).start()

        for c in range(14):
            if c < 12:
                attn_bwd(4 + c)
            cs = slice(c * 256, (c + 1) * 256)
            dh = _dot(df, w2_v[cs, :], _NTD)
            hb = lax.bitcast_convert_type(dhp_v[rows, cs].astype(F32), jnp.int32)
            dhp = jnp.where(hb > 0, dh, jnp.where(hb < 0, 0.5 * dh, 0.0))
            dhp_v[rows, cs] = dhp.astype(BF16)
        return carry

    lax.fori_loop(0, NT, ly, 0)

    C2 = 512

    def dwo_body(c, carry):
        rr = pl.ds(pl.multiple_of(c * C2, C2), C2)
        for u in range(8):
            finalize_pair(8 * c + u)
        wo_v[rr, :] = _dot(oT_v[rr, :], ds_v[...]).astype(BF16)
        pltpu.make_async_copy(wo_v.at[rr, :], dwo_hbm.at[rr, :], out_sems.at[24 + c]).start()
        return carry

    lax.fori_loop(0, D // C2, dwo_body, 0)

    dxs_v = gate_v

    def ln_stats(dxnT, xnT):
        m1 = jnp.mean(dxnT, axis=0, keepdims=True)
        m2 = jnp.mean(dxnT * xnT, axis=0, keepdims=True)
        return m1, m2

    def ln_bwd_chunk(rows, cols, n, dxnT, m1, m2):
        u = dxnT - m1 - xnT_v[cols, rows].astype(F32) * m2
        dx = dy_v[rows, cols].astype(F32) + jnp.tile(rstd_v[rows, :], (1, n // 128)) * u.T
        dxs_v[rows, cols] = dx.astype(BF16)

    def p3(t, carry):
        rows = pl.ds(pl.multiple_of(t * T, T), T)
        rp = pl.ds(pl.multiple_of(jnp.maximum(t - 1, 0) * T, T), T)
        never = _never(t)
        prev = dxn_v[...]
        bq = _dot(wall_v[:, 0:D], phiq_v[:, 0:64, rows].reshape(D, T))
        m1, m2 = ln_stats(_tie(never, bq, prev), xnT_v[:, rp].astype(F32))
        dhp_t = dhp_v[rows, :]
        dpk = []
        dv = []
        bigs = []
        for c in range(8):
            for p in (2 * c, 2 * c + 1):
                phk = phik_v[p, :, rows]
                rhs = jnp.concatenate([vT_v[p * 64:(p + 1) * 64, rows], ones_rows, zrows], axis=0)
                dphi = _dot(at_v[p], rhs)
                dpk.append(_softmax_pm_bwd(phk.astype(F32), dphi).astype(BF16))
                dv.append(_dot(abf_v[p, 0:64, :], phk).astype(BF16))
            cs = slice(c * 128, (c + 1) * 128)
            bigs.append(_dot(w1_v[cs, :], dhp_t, _NTD))
            ln_bwd_chunk(rp, cs, 128, _tie(never, bigs[c], prev[cs]), m1, m2)
        big = jnp.concatenate(bigs, axis=0)
        dpkT = jnp.concatenate(dpk, axis=0)
        dvT = jnp.concatenate(dv, axis=0)
        phik_v[:, 0:64, rows] = dpkT.reshape(NP, 64, T)
        vT_v[:, rows] = dvT
        dxn_v[...] = big + bq + _dot(wall_v[:, 2 * D:3 * D], dvT) + _dot(wall_v[:, D:2 * D], dpkT)

        @pl.when(t > 0)
        def _():
            pltpu.make_async_copy(dxs_v.at[rp, :], dx_hbm.at[rp, :], out_sems.at[8 + t - 1]).start()

        return carry

    lax.fori_loop(0, NT, p3, 0)
    rl = pl.ds((NT - 1) * T, T)
    m1l, m2l = ln_stats(dxn_v[...], xnT_v[:, rl].astype(F32))
    st_v[0:8, :] = jnp.broadcast_to(m1l, (8, T))
    st_v[8:16, :] = jnp.broadcast_to(m2l, (8, T))

    C1 = 256

    def dw1_body(c, carry):
        rr = pl.ds(pl.multiple_of(c * C1, C1), C1)
        never = _never(c)
        res = _dot(xnT_v[rr, :], dhp_v[...])
        ln_bwd_chunk(rl, rr, C1, _tie(never, res[:, 0:T], dxn_v[rr, :]), st_v[0:1, :], st_v[8:9, :])
        w1_v[rr, :] = res.astype(BF16)
        pltpu.make_async_copy(w1_v.at[rr, :], dw1_hbm.at[rr, :], out_sems.at[26 + c]).start()
        return carry

    lax.fori_loop(0, D // C1, dw1_body, 0)
    pltpu.make_async_copy(dxs_v.at[rl, :], dx_hbm.at[rl, :], out_sems.at[8 + NT - 1]).start()

    cp_wq.wait()
    cp_wk.wait()

    CG = 128
    CF = F // 8

    def g_body(c, carry):
        rr = pl.ds(pl.multiple_of(c * CG, CG), CG)
        rk = pl.ds(pl.multiple_of(D + c * CG, CG), CG)
        r2 = pl.ds(pl.multiple_of(c * CF, 64), CF)
        w2_v[r2, :] = _dot(hT_v[r2, :], df_v[...]).astype(BF16)
        pltpu.make_async_copy(w2_v.at[r2, :], dw2_hbm.at[r2, :], out_sems.at[16 + c]).start()
        xr = xnT_v[rr, :]
        gq = _dot(xr, phiq_v[:, 0:64, :].reshape(D, S), _NTD).astype(BF16)
        gk = _dot(xr, phik_v[:, 0:64, :].reshape(D, S), _NTD).astype(BF16)
        wqk = jnp.concatenate([wt_v[rr, :], wt_v[rk, :]], axis=0)
        for g in range(8):
            cg = slice(g * 128, (g + 1) * 128)
            wb = wbd_v[cg, :]
            wall_v[rr, cg] = _dot(gq[:, cg], wb, _NTD).astype(BF16)
            wall_v[rr, D + g * 128:D + (g + 1) * 128] = _dot(gk[:, cg], wb, _NTD).astype(BF16)
            m_v[g] += _dot(wqk[:, cg], jnp.concatenate([gq[:, cg], gk[:, cg]], axis=0), _TN)
        pltpu.make_async_copy(wall_v.at[rr, 0:2 * D], dwqkv_hbm.at[rr, 0:2 * D], out_sems.at[30 + c]).start()
        wall_v[rr, 2 * D:3 * D] = _dot(xr, vT_v[...], _NTD).astype(BF16)
        pltpu.make_async_copy(wall_v.at[rr, 2 * D:3 * D], dwqkv_hbm.at[rr, 2 * D:3 * D], out_sems.at[38 + c]).start()
        return carry

    lax.fori_loop(0, D // CG, g_body, 0)

    for g in range(8):
        mb = jnp.where(bmask, m_v[g], 0.0).astype(BF16)
        wphi_ref[g * 128:(g + 1) * 128, :] = _dot(mb, expand, _NTD).astype(BF16)
    cp_dwphi = pltpu.make_async_copy(wphi_ref, dwphi_hbm, in_sems.at[1])
    cp_dwphi.start()

    for t in range(NT):
        rows = pl.ds(t * T, T)
        pltpu.make_async_copy(x_v.at[rows, :], out_hbm.at[rows, :], out_sems.at[t]).wait()
        pltpu.make_async_copy(dxs_v.at[rows, :], dx_hbm.at[rows, :], out_sems.at[8 + t]).wait()
    for c in range(8):
        rr = pl.ds(c * CF, CF)
        pltpu.make_async_copy(w2_v.at[rr, :], dw2_hbm.at[rr, :], out_sems.at[16 + c]).wait()
    for c in range(D // C2):
        rr = pl.ds(c * C2, C2)
        pltpu.make_async_copy(wo_v.at[rr, :], dwo_hbm.at[rr, :], out_sems.at[24 + c]).wait()
    for c in range(D // C1):
        rr = pl.ds(c * C1, C1)
        pltpu.make_async_copy(w1_v.at[rr, :], dw1_hbm.at[rr, :], out_sems.at[26 + c]).wait()
    for c in range(D // CG):
        rr = pl.ds(c * CG, CG)
        pltpu.make_async_copy(wall_v.at[rr, 0:2 * D], dwqkv_hbm.at[rr, 0:2 * D], out_sems.at[30 + c]).wait()
        pltpu.make_async_copy(wall_v.at[rr, 2 * D:3 * D], dwqkv_hbm.at[rr, 2 * D:3 * D], out_sems.at[38 + c]).wait()
    cp_dwphi.wait()


@jax.jit
def pallas_recurrent_scan__linear_kernel_hedgehog__dense_activation_relu__prompt_kernel(
    A_x: jax.Array,
    A_wqkv: jax.Array,
    A_w_phi: jax.Array,
    A_wo: jax.Array,
    B_x: jax.Array,
    B_w1: jax.Array,
    B_w2: jax.Array,
    grad_out: jax.Array,
):
    del B_x
    x = A_x.reshape(S, D)
    dy = grad_out.reshape(S, D)
    wphi = A_w_phi.reshape(H * DH, DH)
    any_spec = pl.BlockSpec(memory_space=pl.ANY)
    out_shape = (
        jax.ShapeDtypeStruct((S, D), BF16),
        jax.ShapeDtypeStruct((S, D), BF16),
        jax.ShapeDtypeStruct((D, 3 * D), BF16),
        jax.ShapeDtypeStruct((H * DH, DH), BF16),
        jax.ShapeDtypeStruct((D, D), BF16),
        jax.ShapeDtypeStruct((D, F), BF16),
        jax.ShapeDtypeStruct((F, D), BF16),
    )
    scratch = [
        pltpu.VMEM((S, D), BF16),
        pltpu.VMEM((S, D), BF16),
        pltpu.VMEM((D, 3 * D), BF16),
        pltpu.VMEM((3 * D, D), BF16),
        pltpu.VMEM((D, D), BF16),
        pltpu.VMEM((D, F), BF16),
        pltpu.VMEM((F, D), BF16),
        pltpu.VMEM((D, 128), BF16),
        pltpu.VMEM((D, S), BF16),
        pltpu.VMEM((S, 128), F32),
        pltpu.VMEM((NP, 128, S), BF16),
        pltpu.VMEM((NP, 128, S), BF16),
        pltpu.VMEM((D, S), BF16),
        pltpu.VMEM((F, S), BF16),
        pltpu.VMEM((S, F), BF16),
        pltpu.VMEM((S, D), BF16),
        pltpu.VMEM((D, S), BF16),
        pltpu.VMEM((S, D), BF16),
        pltpu.VMEM((S, D), BF16),
        pltpu.VMEM((NP, AR, 128), F32),
        pltpu.VMEM((NP, AR, 128), BF16),
        pltpu.VMEM((NP, 128, 128), BF16),
        pltpu.VMEM((8, 128, 128), F32),
        pltpu.VMEM((D, T), F32),
        pltpu.VMEM((16, T), F32),
        pltpu.VMEM((3 * D, T), F32),
        pltpu.VMEM((H * DH, DH), BF16),
        pltpu.SemaphoreType.DMA((9,)),
        pltpu.SemaphoreType.DMA((NT,)),
        pltpu.SemaphoreType.DMA((8,)),
        pltpu.SemaphoreType.DMA((46,)),
    ]
    outs = pl.pallas_call(
        _kernel,
        out_shape=out_shape,
        in_specs=[any_spec] * 7,
        out_specs=(any_spec,) * 7,
        scratch_shapes=scratch,
        compiler_params=pltpu.CompilerParams(vmem_limit_bytes=124 * 1024 * 1024),
    )(x, A_wqkv, wphi, A_wo, B_w1, B_w2, dy)
    out, dx, dwqkv, dwphi, dwo, dw1, dw2 = outs
    return (out.reshape(1, S, D), dx.reshape(1, S, D), dwqkv, dwphi.reshape(H, DH, DH), dwo, dw1, dw2)
```
